```python
import jax
import jax.numpy as jnp

def _softmax(x, axis=-1):
    return jax.nn.softmax(x, axis=axis)
def _gelu(x):
    return jax.nn.gelu(x, approximate=True)
def _silu(x):
    return jax.nn.silu(x)
def _sigmoid(x):
    return jax.nn.sigmoid(x)
def _layernorm(x, axis=-1, eps=1e-5):
    m = jnp.mean(x, axis=axis, keepdims=True)
    v = jnp.var(x, axis=axis, keepdims=True)
    return (x - m) / jnp.sqrt(v + eps)
def _scatter_add(tgt, idx, src, axis=0):
    return tgt.at[idx].add(src)
def _segment_sum(src, seg, n):
    return jax.ops.segment_sum(src, seg, n)
class _Rng:
    def __init__(self, key):
        self._k = key
    def _next(self):
        self._k, sub = jax.random.split(self._k)
        return sub
    def normal(self, shape):
        return jax.random.normal(self._next(), shape, dtype=jnp.bfloat16)
    def randint(self, lo, hi, shape):
        return jax.random.randint(self._next(), shape, lo, hi, dtype=jnp.int32)
    def uniform(self, shape, lo=0.0, hi=1.0):
        return jax.random.uniform(self._next(), shape, jnp.bfloat16, lo, hi)
    def permutation(self, n):
        return jax.random.permutation(self._next(), n)


kernel_name = 'gated_mix__sliding_block_cached__moe_arch_mod__decode'

def setup_inputs():
    _rng = _Rng(jax.random.key(int.from_bytes(__import__("os").urandom(4), "little")))
    _w = (lambda a: (lambda t: t.astype(jnp.bfloat16) if jnp.issubdtype(t.dtype, jnp.floating) else t)(jnp.asarray(a)))
    def _A_setup():
        B, Sq, D = 1, 1, 640
        Hq, Hkv, Sk, Dh = 32, 32, 32768, 192
        assert Hq % Hkv == 0, (Hq, Hkv)
        return {
            "x": _w((lambda *s: _rng.normal(s) * 0.05)(B, Sq, D)),
            "k_cache": _w((lambda *s: _rng.normal(s) * 0.05)(B, Hkv, Sk, Dh)),
            "v_cache": _w((lambda *s: _rng.normal(s) * 0.05)(B, Hkv, Sk, Dh)),
            "wq": _w((lambda *s: _rng.normal(s) * 0.05)(D, Hq * Dh) * (D ** -0.5)),
            "wo": _w((lambda *s: _rng.normal(s) * 0.05)(Hq * Dh, D) * ((Hq * Dh) ** -0.5)),
        }
    _A_in = _A_setup()

    def _B_setup():
        B, S, D, F, C = 1, 1, 640, 1536, 1
        return {
            "x": _w((lambda *s: _rng.normal(s) * 0.05)(B, S, D)),
            "w_r": _w((lambda *s: _rng.normal(s) * 0.05)(D)),
            "w_gate": _w((lambda *s: _rng.normal(s) * 0.05)(D, F)),
            "w_up": _w((lambda *s: _rng.normal(s) * 0.05)(D, F)),
            "w_down": _w((lambda *s: _rng.normal(s) * 0.05)(F, D)),
        }
    _B_in = _B_setup()

    return {
        "A_x": _A_in["x"],
        "A_k_cache": _A_in["k_cache"],
        "A_v_cache": _A_in["v_cache"],
        "A_wq": _A_in["wq"],
        "A_wo": _A_in["wo"],
        "B_x": _B_in["x"],
        "B_w_r": _B_in["w_r"],
        "B_w_gate": _B_in["w_gate"],
        "B_w_up": _B_in["w_up"],
        "B_w_down": _B_in["w_down"],
        "gate_w": _w((lambda *s: _rng.normal(s) * 0.05)(640)),
    }

def reference(A_x, A_k_cache, A_v_cache, A_wq, A_wo, B_x, B_w_r, B_w_gate, B_w_up, B_w_down, gate_w):
    def _A_ref(x, k_cache, v_cache, wq, wo):
        B, Sq, D = x.shape
        Hq, Dh = 32, 192
        Hkv, Sk = k_cache.shape[1], k_cache.shape[2]
        W = min(4096, max(256, Sk // 4))
        rep = Hq // Hkv
        q = (lambda x, *d: x.transpose(*d))((x @ wq).reshape(B, Sq, Hq, Dh), 0, 2, 1, 3)
        k = jnp.repeat(k_cache[:, :, Sk - W:, :], rep, axis=1)
        v = jnp.repeat(v_cache[:, :, Sk - W:, :], rep, axis=1)
        scores = jnp.einsum("bhqd,bhkd->bhqk", q, k) * (Dh ** -0.5)
        p = _softmax(scores, axis=-1)
        o = jnp.einsum("bhqk,bhkd->bhqd", p, v)
        return (lambda x, *d: x.transpose(*d))(o, 0, 2, 1, 3).reshape(B, Sq, Hq * Dh) @ wo

    def _B_ref(x, w_r, w_gate, w_up, w_down):
        B, S, D = x.shape
        C = 1
        r = x @ w_r
        idx = jnp.argsort(-r, axis=-1)[:, :C]
        idx_e = jnp.repeat(idx.reshape(B, C, 1), D, axis=2)
        x_sel = jnp.take_along_axis(x, idx_e, axis=1)
        g = _silu(x_sel @ w_gate)
        u = x_sel @ w_up
        y = (g * u) @ w_down
        r_sel = _sigmoid(jnp.take_along_axis(r, idx, axis=1))
        y = y * r_sel.reshape(B, C, 1)
        b_off = (jnp.arange(B) * S).reshape(B, 1)
        flat_idx = (idx + b_off).reshape(B * C)
        zero = (x * 0.0).reshape(B * S, D)
        upd = _scatter_add(zero, flat_idx, y.reshape(B * C, D), axis=0)
        return x + upd.reshape(B, S, D)

    x = A_x
    g = _sigmoid((x * gate_w).sum(-1, keepdims=True))
    a = _A_ref(x, A_k_cache, A_v_cache, A_wq, A_wo)
    b = _B_ref(x, B_w_r, B_w_gate, B_w_up, B_w_down)
    return g * a + (1 - g) * b
```

```python
import functools
import contextlib
import jax
import jax.numpy as jnp
import jax.experimental.pallas as pl
import jax.experimental.pallas.tpu as pltpu

H, DH, SK, D, F = 32, 192, 32768, 640, 1536
W = min(4096, max(256, SK // 4))
BASE = SK - W
M = 8
f32 = jnp.float32
bf16 = jnp.bfloat16

DEFAULT = dict(
    KR=32, KC=512, HB=96, L=30, BU=16, dpt=7, A=5, lag0=6, dly=50, dly_pre=None, dly_post=None, dly_c=0, rot=1, cmul=1,
    ROWS=15, WR=3, wrot=1, wmul=1, nsem=48, scopes=False, compute=True, G=256,
    dreg=4, TP=32, frot=1, small_at=2, DCH=256, swap=False, ilv=3,
)


def tiles(w, rows):
    r, c = w.shape
    return w.reshape(r // 8, 8, c // 128, 128).transpose(0, 2, 1, 3).reshape(rows, r * c // 128 // rows, 128)


def make(**kw):
    cfg = dict(DEFAULT); cfg.update(kw)
    KR, KC, L, A, NSEM, LAG0, ROWS, WR, HB = (cfg[k] for k in ('KR', 'KC', 'L', 'A', 'nsem', 'lag0', 'ROWS', 'WR', 'HB'))
    NG = W // KC
    NR = HB // KR
    SPP = 2 * DH // KR * NG
    assert SPP % NSEM == 0 and L <= NSEM and A + LAG0 < NSEM
    comp = cfg['compute']
    NP = H // 2
    RING = 3

    def scope(name):
        return jax.named_scope(name) if cfg['scopes'] else contextlib.nullcontext()

    def kernel(x_hbm, kT, vT, wq, wo, wr_hbm, wg, wu, wd, gw_hbm, out_ref,
               x_v, wr_v, gw_v, wq_b, k_b, v_b, wo_b, wg_b, wu_b, wd_b,
               s_s, p_s, hb_s, sem1, sem0, sems):
        small = [pltpu.make_async_copy(x_hbm, x_v, sems.at[0]),
                 pltpu.make_async_copy(gw_hbm, gw_v, sems.at[1]),
                 pltpu.make_async_copy(wr_hbm, wr_v, sems.at[2])]

        def wp(src, dst, idx):
            return lambda sem: pltpu.make_async_copy(src.at[idx], dst.at[idx], sem)

        def kvp(q, hp, slot, j):
            which = q ^ cfg['swap']
            b, j = divmod(j, NR * NG)
            g, r = divmod(j, NR)
            g = ((g + q * cfg['rot']) * cfg['cmul']) % NG
            rows = pl.ds(b * HB + r * KR, KR)
            src = (kT, vT)[which].at[hp, rows, pl.ds(BASE + g * KC, KC)]
            dst = (k_b, v_b)[which].at[slot, rows, pl.ds(g * KC, KC)]
            return lambda sem: pltpu.make_async_copy(src, dst, sem)

        ngrp = ROWS // WR
        ncol = wq.shape[1] // 32
        n_pre = ncol * ngrp
        wdst = (wq_b.reshape(*wq.shape), wo_b.reshape(*wo.shape))

        def pre_piece(which, c, r):
            c = ((c + which * cfg['wrot']) * cfg['wmul']) % ncol
            return wp((wq, wo)[which], wdst[which], (pl.ds(r * WR, WR), pl.ds(c * 32, 32)))

        post = [[], []]
        for which, (src, dst) in enumerate(((wg, wg_b), (wu, wu_b))):
            for c in range(60):
                c = (c + which * cfg['frot']) % 60
                t, cc = divmod(c, 3)
                post[which].append(wp(src, dst, (slice(None), pl.ds(t * 8, 8), pl.ds(cc * 512, 512))))
        nreg, TP = cfg['dreg'], cfg['TP']
        npd = F // TP
        d_pos = {}
        for i in range(npd):
            reg, k = i % nreg, i // nreg
            r0 = (reg * (npd // nreg) + k) * TP
            d_pos[r0] = (i % 2, len(post[i % 2]))
            post[i % 2].append(wp(wd, wd_b, (pl.ds(r0, TP), slice(None))))
        n_post = len(post[0])

        def pace(d):
            if d:
                pl.delay(d)

        deferred = []

        def step(i, piece, has_prev=True, open_loop=False, chunk=None):
            w1 = piece(0, 0)(sem1.at[i % NSEM])
            w0 = piece(1, -LAG0)(sem0.at[(i - LAG0) % NSEM]) if has_prev else None
            if open_loop:
                deferred.extend([w1, w0])
                assert len(deferred) // 2 + L <= NSEM
            else:
                for w in deferred:
                    w.wait()
                deferred.clear()
                if w0 is not None:
                    w0.wait()
                w1.wait()
            p = piece(1, A)
            if p is not None:
                p(sem0.at[(i + A) % NSEM]).start(priority=0)
            p = piece(0, L)
            if p is not None:
                p(sem1.at[(i + L) % NSEM]).start(priority=1)

        def pre_at(q, pos):
            if pos >= n_pre:
                return kvp(q, 0, 0, pos - n_pre)
            return pre_piece(q, pos // ngrp, pos % ngrp)

        dly_pre = cfg['dly_pre'] if cfg['dly_pre'] is not None else 12 * WR
        with scope("zz_pre"):
            ilv = cfg['ilv']
            for i in range(L):
                if i == cfg['small_at']:
                    for c in small:
                        c.start()
                pre_at(0, i)(sem1.at[(i - n_pre) % NSEM]).start(priority=1)
                if i % ilv == 0 and i // ilv < A:
                    pre_at(1, i // ilv)(sem0.at[(i // ilv - n_pre) % NSEM]).start(priority=0)
            for i in range((L + ilv - 1) // ilv, A):
                pre_at(1, i)(sem0.at[(i - n_pre) % NSEM]).start(priority=0)
            for i in range(n_pre):
                step(i - n_pre, lambda q, k: pre_at(q, i + k), has_prev=i >= LAG0)
                if i == 40:
                    for c in small:
                        c.wait()
                    x = x_v[0]
                    xf = x.astype(f32)
                    gate = jax.nn.sigmoid(jnp.sum(xf * gw_v[...].astype(f32).reshape(1, D), axis=-1, keepdims=True))
                    rsel = jax.nn.sigmoid(jnp.sum(xf * wr_v[...].astype(f32).reshape(1, D), axis=-1, keepdims=True))
                    xm = jnp.broadcast_to(x, (M, D))
                else:
                    pace(dly_pre)

        scale = DH ** -0.5
        G = cfg['G']
        NTG = W // G

        def pair_tasks(hp, slot, st):
            def t_q(c):
                w = wq_b[:, pl.ds(pl.multiple_of((3 * hp + c) * 8, 8), 8), :].reshape(D, 128)
                st['q', c] = jnp.dot(xm, w, preferred_element_type=f32)
                if c == 2:
                    q = jnp.concatenate([st['q', k] for k in range(3)], axis=1)
                    row = jax.lax.broadcasted_iota(jnp.int32, (M, 2 * DH), 0)
                    col = jax.lax.broadcasted_iota(jnp.int32, (M, 2 * DH), 1)
                    st['own'] = (row >= M // 2) == (col >= DH)
                    st['q'] = jnp.where(st['own'], q, 0.0).astype(bf16)

            def t_qk(g):
                sl = slice(g * G, (g + 1) * G)
                st['s', g] = jnp.dot(st['q'], k_b[slot, :, sl], preferred_element_type=f32) * scale
                if (g + 1) % BU == 0:
                    for k in range(g + 1 - BU, g + 1):
                        sc = st['s', k]
                        s_s[:, k * G:(k + 1) * G] = sc
                        for t in range(G // 128):
                            v = sc[:, t * 128:(t + 1) * 128]
                            st['m'] = v if k == 0 and t == 0 else jnp.maximum(st['m'], v)

            def t_max():
                st['m'] = jnp.max(st['m'], axis=-1, keepdims=True)

            def t_exp():
                e = jnp.exp(s_s[...] - st['m'])
                p_s[...] = e
                st['l'] = jnp.sum(e, axis=-1, keepdims=True)

            def t_pv(g):
                sl = slice(g * G, (g + 1) * G)
                if g == 0:
                    st['inv'] = 1.0 / st['l']
                r = jax.lax.dot_general((p_s[:, sl] * st['inv']).astype(bf16), v_b[slot, :, sl],
                                        (((1,), (1,)), ((), ())), preferred_element_type=f32)
                st['acc'] = r if g == 0 else st['acc'] + r

            def t_o(k):
                if k == 0:
                    st['o'] = jnp.where(st['own'], st['acc'], 0.0).astype(bf16)
                rows = pl.ds(hp * 24 + k * 8, 8)
                w = jnp.concatenate(
                    [jnp.concatenate([wo_b[rows, c * 8:c * 8 + 8, :], wo_b[rows, 40 + c * 8:48 + c * 8, :]], axis=1)
                     .reshape(128, 128) for c in range(5)], axis=1)
                st['a'] = st['a'] + jnp.dot(st['o'][:, k * 128:(k + 1) * 128], w, preferred_element_type=f32)
            P = functools.partial
            return ([[P(t_q, c) for c in range(3)]] + [[P(t_qk, g + k) for k in range(BU)] for g in range(0, NTG, BU)]
                    + [[t_max], [t_exp]]
                    + [[P(t_pv, g + k) for k in range(BU)] for g in range(0, NTG, BU)] + [[P(t_o, k) for k in range(3)]])

        BU = cfg['BU']

        def spread(bursts, lo, hi):
            out = {}
            gap = (hi - lo - sum(len(b) for b in bursts)) / len(bursts)
            assert gap >= 0
            n = 0
            for k, b in enumerate(bursts):
                i = lo + int(k * gap) + n
                for j, t in enumerate(b):
                    out[i + j] = (t, j > 0)
                n += len(b)
            return out

        def full_step(tasks, i, piece, d):
            t, cont = tasks.get(i, (None, False)) if comp else (None, False)
            step(i, piece, open_loop=cont)
            if t is not None:
                t()
            else:
                pace(d)

        def pair(hp, slots, tasks, first=False, last=False):
            def at(q, pos):
                if pos < 0:
                    return pre_at(q, n_pre + pos) if first else kvp(q, hp - 1, slots[0], pos + SPP)
                if pos >= SPP:
                    return post[q][pos - SPP] if last else kvp(q, hp + 1, slots[2], pos - SPP)
                return kvp(q, hp, slots[1], pos)
            for i in range(SPP):
                full_step(tasks, i, lambda q, k: at(q, i + k), cfg['dly'])
            assert not deferred

        with scope("zz_h0"):
            pair(0, (2, 0, 1), {}, first=True)

        def body(hp, carry):
            a, s0, s1, s2 = carry
            st = dict(a=a)
            pair(hp, (s0, s1, s2), spread(pair_tasks(hp - 1, s0, st), LAG0, SPP))
            return st['a'], s1, s2, s0

        with scope("zz_loop"):
            a = jax.lax.fori_loop(1, NP - 1, body, (jnp.zeros((M, D), f32), 0, 1, 2))[0]
        st = dict(a=a)
        with scope("zz_h31"):
            pair(NP - 1, ((NP - 2) % 3, (NP - 1) % 3, None), spread(pair_tasks(NP - 2, (NP - 2) % 3, st), LAG0, SPP), last=True)

        GC = 128

        def t_gu(src, key, cb):
            w = src[:, :, cb * GC:(cb + 1) * GC].reshape(D, GC)
            st[key, cb] = jnp.dot(xm, w, preferred_element_type=f32)

        def t_h(j):
            hj = (jax.nn.silu(st['g', j]) * st['u', j]).astype(bf16).astype(f32)
            hb_s[j * 128:(j + 1) * 128, :] = jnp.broadcast_to(hj[0:1], (128, 128)).T

        def t_d(r0):
            w = wd_b[r0:r0 + TP, :].astype(f32)
            hb = hb_s[r0:r0 + TP, :]
            for k in range(TP // 8):
                rows = slice(k * 8, k * 8 + 8)
                part = w[rows] * jnp.concatenate([hb[rows]] * 5, axis=1)
                st['y'] = st['y'] + part if 'y' in st else part

        P = functools.partial
        tasks = spread(pair_tasks(NP - 1, (NP - 1) % 3, st), LAG0, 59)
        both = lambda *fs: (lambda: [f() for f in fs])
        for k in range(6):
            tasks[59 + k] = (both(*[P(t_gu, wg_b, 'g', 2 * k + j) for j in range(2)]), k > 0)
            tasks[66 + k] = (both(*[P(t_gu, wu_b, 'u', 2 * k + j) for j in range(2)]), k > 0)
        for k in range(3):
            tasks[73 + k] = (both(*[P(t_h, 4 * k + j) for j in range(4)]), k > 0)
        todo = sorted((pos + LAG0 * q, r0) for r0, (q, pos) in d_pos.items())
        for i in range(76, n_post):
            now = [r0 for rdy, r0 in todo if rdy <= i][:cfg['dpt']]
            todo = [t for t in todo if t[1] not in now]
            if now:
                tasks[i] = (both(*[P(t_d, r0) for r0 in now]), False)

        def post_at(q, pos):
            if pos < 0:
                return kvp(q, NP - 1, (NP - 1) % 3, pos + SPP)
            return post[q][pos] if pos < n_post else None

        dly_post = cfg['dly_post'] if cfg['dly_post'] is not None else cfg['dly']
        with scope("zz_post"):
            for i in range(n_post):
                full_step(tasks, i, lambda q, k: post_at(q, i + k), dly_post if i + A < n_post - 1 else 0)
        with scope("zz_tail"):
            for i in range(n_post, n_post + LAG0):
                post[1][i - LAG0](sem0.at[(i - LAG0) % NSEM]).wait()
                for rdy, r0 in todo:
                    if max(rdy, n_post) == i and comp:
                        t_d(r0)
            if comp:
                a = st['a'][0:1] + st['a'][M // 2:M // 2 + 1]
                y = jnp.sum(st['y'], axis=0, keepdims=True)
                b = xf + (xf * 0.0 + y * rsel)
                out_ref[0] = (gate * a + (1.0 - gate) * b).astype(bf16)
            else:
                out_ref[0] = (xf * gate * rsel).astype(bf16)

    def fn(A_x, A_k_cache, A_v_cache, A_wq, A_wo, B_x, B_w_r, B_w_gate, B_w_up, B_w_down, gate_w):
        del B_x
        kT = jnp.swapaxes(A_k_cache, 2, 3).reshape(NP, 2 * DH, SK)
        vT = jnp.swapaxes(A_v_cache, 2, 3).reshape(NP, 2 * DH, SK)
        any_spec = pl.BlockSpec(memory_space=pl.ANY)
        vmem = pltpu.VMEM
        return pl.pallas_call(
            kernel,
            out_shape=jax.ShapeDtypeStruct((1, 1, D), bf16),
            in_specs=[any_spec] * 10,
            out_specs=pl.BlockSpec(memory_space=pltpu.VMEM),
            scratch_shapes=[
                vmem((1, 1, D), bf16), vmem((D,), bf16), vmem((D,), bf16),
                vmem((80, 384, 128), bf16), vmem((RING, 2 * DH, W), bf16), vmem((RING, 2 * DH, W), bf16),
                vmem((384, 80, 128), bf16), vmem((4, D // 4, F), bf16), vmem((4, D // 4, F), bf16),
                vmem((F, D), bf16),
                vmem((M, W), f32), vmem((M, W), f32), vmem((F, 128), f32),
                pltpu.SemaphoreType.DMA((NSEM,)), pltpu.SemaphoreType.DMA((NSEM,)),
                pltpu.SemaphoreType.DMA((3,)),
            ],
            compiler_params=pltpu.CompilerParams(
                vmem_limit_bytes=64 * 1024 * 1024,
                disable_semaphore_checks=True, disable_bounds_checks=True,
            ),
            name="gated_mix_decode",
        )(A_x, kT, vT, tiles(A_wq, ROWS), tiles(A_wo, ROWS), B_w_r,
          B_w_gate.reshape(4, D // 4, F), B_w_up.reshape(4, D // 4, F), B_w_down, gate_w)
    return fn


_fn = make()


@jax.jit
def pallas_gated_mix__sliding_block_cached__moe_arch_mod__decode_kernel(
        A_x, A_k_cache, A_v_cache, A_wq, A_wo, B_x, B_w_r, B_w_gate, B_w_up, B_w_down, gate_w):
    return _fn(A_x, A_k_cache, A_v_cache, A_wq, A_wo, B_x, B_w_r, B_w_gate, B_w_up, B_w_down, gate_w)
```

```python
import functools
import contextlib
import jax
import jax.numpy as jnp
import jax.experimental.pallas as pl
import jax.experimental.pallas.tpu as pltpu

H, DH, SK, D, F = 32, 192, 32768, 640, 1536
W = min(4096, max(256, SK // 4))
BASE = SK - W
M = 8
NP = H // 2
f32 = jnp.float32
bf16 = jnp.bfloat16


def sweep(txt, ncol, off=None):
    split, pos = [], {}
    for t in txt.split():
        k, n = t[0], int(t[1:])
        split.append((k, pos.get(k, 0), n)); pos[k] = pos.get(k, 0) + n
    return [(k, r0, n, (c + (off or {}).get(k, 0)) % ncol[k], 1)
            for c in range(max(ncol[k] for k, _, _ in split)) for k, r0, n in split if c < ncol[k]]


def kvseq(kt, vt=None):
    vt = vt or kt
    return [(a, h * 24 + r0, n, c, nc) for a, t in (('k', kt), ('v', vt)) for h in range(2) for _, r0, n, c, nc in t]


NC = dict(q=64, o=64, g=60, u=60, d=60, k=8)
DEFAULT = dict(
    kv=kvseq(sweep("k4 k2 " * 4, NC)), L=30, A=11, lag0=4, dly=0, dly0=0, dly_w=0,
    pre=sweep("q4 q2 q4 q2 q3 g2 g2 u2 d4 u2", NC, dict(g=1, u=1, d=1)), post=sweep("o3 o3 o3 o3 o3", NC),
    nsem=64, scopes=False, compute=True, G=256, BU=8, dpt=4, n_att=64, small_at=10,
)


def tiles(w, rows):
    r, c = w.shape
    return w.reshape(r // 8, 8, c // 128, 128).transpose(0, 2, 1, 3).reshape(rows, r * c // 1024 // rows, 8, 128)


def make(**kw):
    cfg = dict(DEFAULT); cfg.update(kw)
    L, A, NSEM, LAG0 = (cfg[k] for k in ('L', 'A', 'nsem', 'lag0'))
    SPP = len(cfg['kv']) // 2
    assert SPP % NSEM == 0 and L <= NSEM and A + LAG0 < NSEM
    comp = cfg['compute']

    def scope(name):
        return jax.named_scope(name) if cfg['scopes'] else contextlib.nullcontext()

    def kernel(x_hbm, kT, vT, wq, wo, wr_hbm, wg, wu, wd, gw_hbm, out_ref,
               x_v, wr_v, gw_v, wq_b, k_b, v_b, wo_b, wg_b, wu_b, wd_b,
               q_s, s_s, ob_s, sem1, sem0, sems):
        small = [pltpu.make_async_copy(x_hbm, x_v, sems.at[0]),
                 pltpu.make_async_copy(gw_hbm, gw_v, sems.at[1]),
                 pltpu.make_async_copy(wr_hbm, wr_v, sems.at[2])]

        def kvp(q, hp, slot, j):
            a, r0, n, c, nc = cfg['kv'][2 * j + q]
            rows = pl.ds(r0 * 8, n * 8)
            src = dict(k=kT, v=vT)[a].at[hp, rows, pl.ds(BASE + c * 512, nc * 512)]
            dst = dict(k=k_b, v=v_b)[a].at[slot, rows, pl.ds(c * 512, nc * 512)]
            return lambda sem: pltpu.make_async_copy(src, dst, sem)

        bufs = dict(q=(wq, wq_b), o=(wo, wo_b), g=(wg, wg_b), u=(wu, wu_b), d=(wd, wd_b))

        def wpiece(k, r0, n, c, nc):
            idx = (pl.ds(r0, n), pl.ds(c * 4, nc * 4))
            return lambda sem: pltpu.make_async_copy(bufs[k][0].at[idx], bufs[k][1].at[idx], sem)

        pre = [wpiece(*p) for p in cfg['pre']]
        post = [wpiece(*p) for p in cfg['post']]
        assert len(pre) % 2 == 0 and len(post) % 2 == 0
        n_pre, n_post = len(pre) // 2, len(post) // 2

        def pace(d):
            if d:
                pl.delay(d)

        deferred = []

        def step(i, piece, has_prev=True, open_loop=False):
            w1 = piece(0, 0)(sem1.at[i % NSEM])
            w0 = piece(1, -LAG0)(sem0.at[(i - LAG0) % NSEM]) if has_prev else None
            if open_loop:
                deferred.extend([w1, w0])
                assert len(deferred) // 2 + L <= NSEM
            else:
                for w in deferred:
                    w.wait()
                deferred.clear()
                if w0 is not None:
                    w0.wait()
                w1.wait()
            p = piece(1, A)
            if p is not None:
                p(sem0.at[(i + A) % NSEM]).start(priority=0)
            p = piece(0, L)
            if p is not None:
                p(sem1.at[(i + L) % NSEM]).start(priority=1)

        def pre_at(q, pos):
            if pos >= n_pre:
                return kvp(q, 0, 0, pos - n_pre)
            return pre[2 * pos + q]

        with scope("zz_pre"):
            per = -(-L // A)
            if cfg.get('st'):
                for i in range(L):
                    pre_at(0, i)(sem1.at[(i - n_pre) % NSEM]).start(priority=1)
                    if i < A:
                        pre_at(1, i)(sem0.at[(i - n_pre) % NSEM]).start(priority=0 if i in cfg['st'] else 1)
            for k in range(0 if cfg.get('st') else A):
                for i in range(k * per, min(L, (k + 1) * per)):
                    pre_at(0, i)(sem1.at[(i - n_pre) % NSEM]).start(priority=1)
                pre_at(1, k)(sem0.at[(k - n_pre) % NSEM]).start(priority=0)
                pace(cfg['dly0'])
            for i in range(n_pre):
                step(i - n_pre, lambda q, k: pre_at(q, i + k), has_prev=i >= LAG0)
                if i == cfg['small_at']:
                    for c in small:
                        c.start()
                if i == 40:
                    for c in small:
                        c.wait()
                    x = x_v[0]
                    xf = x.astype(f32)
                    gate = jax.nn.sigmoid(jnp.sum(xf * gw_v[...].astype(f32).reshape(1, D), axis=-1, keepdims=True))
                    rsel = jax.nn.sigmoid(jnp.sum(xf * wr_v[...].astype(f32).reshape(1, D), axis=-1, keepdims=True))
                    xm = jnp.broadcast_to(x, (M, D))
                else:
                    pace(cfg['dly'])

        def gather(buf, first, n, stride):
            per = buf.shape[1]
            parts, t = [], first
            while n:
                r, o = divmod(t, per)
                m = min(n, -(-(per - o) // stride))
                parts.append(buf[r, pl.ds(o, m, stride=stride)] if m > 1 else buf[r, pl.ds(o, 1)])
                t, n = t + m * stride, n - m
            v = parts[0] if len(parts) == 1 else jnp.concatenate(parts, axis=0)
            return v.reshape(v.shape[0] * 8, 128)

        scale = DH ** -0.5
        G, BU = cfg['G'], cfg['BU']
        NTG = W // G
        P = functools.partial

        def pair_tasks(hp, slot):
            st = {}

            def t_qk(g):
                if g == 0:
                    row = jax.lax.broadcasted_iota(jnp.int32, (M, 2 * DH), 0)
                    col = jax.lax.broadcasted_iota(jnp.int32, (M, 2 * DH), 1)
                    st['own'] = (row >= M // 2) == (col >= DH)
                    st['q'] = jnp.where(st['own'], q_s[hp], 0.0).astype(bf16)
                st['s', g] = jnp.dot(st['q'], k_b[slot, :, g * G:(g + 1) * G], preferred_element_type=f32) * scale
                if (g + 1) % BU == 0:
                    for k in range(g + 1 - BU, g + 1):
                        sc = st['s', k]
                        s_s[:, k * G:(k + 1) * G] = sc
                        for t in range(G // 128):
                            v = sc[:, t * 128:(t + 1) * 128]
                            st['m'] = v if k == 0 and t == 0 else jnp.maximum(st['m'], v)

            def t_max():
                st['m'] = jnp.max(st['m'], axis=-1, keepdims=True)

            def t_exp():
                e = jnp.exp(s_s[...] - st['m'])
                s_s[...] = e
                l = e[:, 0:128]
                for t in range(1, W // 128):
                    l = l + e[:, t * 128:(t + 1) * 128]
                st['l'] = l

            def t_pv(g):
                sl = slice(g * G, (g + 1) * G)
                if g == 0:
                    st['l'] = jnp.sum(st['l'], axis=-1, keepdims=True)
                r = jax.lax.dot_general(s_s[:, sl].astype(bf16), v_b[slot, :, sl],
                                        (((1,), (1,)), ((), ())), preferred_element_type=f32)
                st['acc'] = r if g == 0 else st['acc'] + r

            def t_o(k):
                if k == 0:
                    o = jnp.where(st['own'], st['acc'] / st['l'], 0.0).astype(bf16).astype(f32)
                    st['o'] = o[0:1] + o[M // 2:M // 2 + 1]
                ob_s[hp, k * 128:(k + 1) * 128, :] = jnp.broadcast_to(st['o'][:, k * 128:(k + 1) * 128], (128, 128)).T
            return ([[P(t_qk, g + k) for k in range(BU)] for g in range(0, NTG, BU)] + [[t_max], [t_exp]]
                    + [[P(t_pv, g + k) for k in range(BU)] for g in range(0, NTG, BU)] + [[P(t_o, k) for k in range(3)]])

        def spread(bursts, lo, hi):
            out = {}
            gap = (hi - lo - sum(len(b) for b in bursts)) / len(bursts)
            assert gap >= 1
            n = 0
            for k, b in enumerate(bursts):
                i = lo + int(k * gap) + n
                for j, t in enumerate(b):
                    out[i + j] = (t, j > 0)
                n += len(b)
            return out

        def full_step(tasks, i, piece):
            t, cont = tasks.get(i, (None, False)) if comp else (None, False)
            step(i, piece, open_loop=cont)
            if t is not None:
                t()
                if cont is None:
                    pace(cfg['dly_w'])
            else:
                pace(cfg['dly'])

        def pair(hp, slots, tasks, first=False, last=False):
            def at(q, pos):
                if pos < 0:
                    return pre_at(q, n_pre + pos) if first else kvp(q, hp - 1, slots[0], pos + SPP)
                if pos >= SPP:
                    return post[2 * (pos - SPP) + q] if last else kvp(q, hp + 1, slots[2], pos - SPP)
                return kvp(q, hp, slots[1], pos)
            for i in range(SPP):
                full_step(tasks, i, lambda q, k: at(q, i + k))
            assert not deferred

        ffn = {}

        def t_proj(src, key, cb, nt):
            ffn[key, cb] = jnp.dot(xm, gather(src, cb, D // 8, nt), preferred_element_type=f32)
            if key == 'q' and (cb + 1) % 12 == 0:
                for k in range(cb - 11, cb + 1):
                    q_s[k // 3, :, (k % 3) * 128:(k % 3 + 1) * 128] = ffn['q', k]

        def t_d(j):
            hj = (jax.nn.silu(ffn['g', j]) * ffn['u', j]).astype(bf16)
            w = jnp.concatenate([gather(wd_b, j * 80 + c, 16, 5) for c in range(5)], axis=1)
            r = jnp.dot(hj, w, preferred_element_type=f32)
            ffn['y'] = r if j == 0 else ffn['y'] + r

        def t_b():
            ffn['b'] = (1.0 - gate) * (xf + (xf * 0.0 + ffn['y'][0:1] * rsel))

        with scope("zz_h0"):
            pair(0, (2, 0, 1), spread([[P(t_proj, wq_b, 'q', b + j, 48) for j in range(12)] for b in range(0, 48, 12)]
                                      + [[P(t_proj, wg_b, 'g', j, 12) for j in range(12)], [P(t_proj, wu_b, 'u', j, 12) for j in range(12)],
                                         [P(t_d, j) for j in range(12)], [t_b]], LAG0, SPP), first=True)

        def body(hp, carry):
            s0, s1, s2 = carry
            pair(hp, (s0, s1, s2), spread(pair_tasks(hp - 1, s0), LAG0, SPP))
            return s1, s2, s0

        with scope("zz_loop"):
            jax.lax.fori_loop(1, NP - 1, body, (0, 1, 2))
        with scope("zz_h31"):
            pair(NP - 1, ((NP - 2) % 3, (NP - 1) % 3, None), spread(pair_tasks(NP - 2, (NP - 2) % 3), LAG0, SPP), last=True)

        acc = {}

        def t_wo(pieces):
            for j in pieces:
                _, r0, n, c, nc = cfg['post'][j]
                for r in range(r0, r0 + n):
                    w = wo_b[r, c * 4:(c + nc) * 4].astype(f32)
                    for t in range(4 * nc):
                        kt, ct = divmod(r * 256 + c * 4 + t, 5)
                        part = w[t] * ob_s[kt // 48, (kt % 48) * 8:(kt % 48) * 8 + 8, :]
                        acc[ct] = acc[ct] + part if ct in acc else part

        n_att = cfg['n_att']
        tasks = spread(pair_tasks(NP - 1, (NP - 1) % 3), LAG0, n_att)
        n_main = n_post - A
        done = 0
        for i in range(n_att, n_main):
            upto = min(2 * (i - LAG0 + 1), done + cfg['dpt'])
            tasks[i] = (P(t_wo, range(done, upto)), None)
            done = upto

        def post_at(q, pos):
            if pos < 0:
                return kvp(q, NP - 1, (NP - 1) % 3, pos + SPP)
            return post[2 * pos + q] if pos < n_post else None

        with scope("zz_post"):
            for i in range(n_main):
                full_step(tasks, i, lambda q, k: post_at(q, i + k))
        assert done == 2 * (n_main - LAG0)
        with scope("zz_tail"):
            for j in range(done, 2 * n_post):
                i, q = divmod(j, 2)
                if q or i >= n_main:
                    post[j]((sem1, sem0)[q].at[i % NSEM]).wait()
                if comp:
                    t_wo([j])
            if comp:
                a = jnp.sum(jnp.concatenate([acc[c] for c in range(5)], axis=1), axis=0, keepdims=True)
                out_ref[0] = (gate * a + ffn['b']).astype(bf16)
            else:
                out_ref[0] = (xf * gate * rsel).astype(bf16)

    def fn(A_x, A_k_cache, A_v_cache, A_wq, A_wo, B_x, B_w_r, B_w_gate, B_w_up, B_w_down, gate_w):
        del B_x
        kT = jnp.swapaxes(A_k_cache, 2, 3).reshape(NP, 2 * DH, SK)
        vT = jnp.swapaxes(A_v_cache, 2, 3).reshape(NP, 2 * DH, SK)
        any_spec = pl.BlockSpec(memory_space=pl.ANY)
        vmem = pltpu.VMEM
        big, ffn = vmem((15, 256, 8, 128), bf16), vmem((4, 240, 8, 128), bf16)
        return pl.pallas_call(
            kernel,
            out_shape=jax.ShapeDtypeStruct((1, 1, D), bf16),
            in_specs=[any_spec] * 10,
            out_specs=pl.BlockSpec(memory_space=pltpu.VMEM),
            scratch_shapes=[
                vmem((1, 1, D), bf16), vmem((D,), bf16), vmem((D,), bf16),
                big, vmem((3, 2 * DH, W), bf16), vmem((3, 2 * DH, W), bf16), big, ffn, ffn, ffn,
                vmem((NP, M, 2 * DH), f32), vmem((M, W), f32), vmem((NP, 2 * DH, 128), f32),
                pltpu.SemaphoreType.DMA((NSEM,)), pltpu.SemaphoreType.DMA((NSEM,)),
                pltpu.SemaphoreType.DMA((3,)),
            ],
            compiler_params=pltpu.CompilerParams(
                vmem_limit_bytes=64 * 1024 * 1024,
                disable_semaphore_checks=True, disable_bounds_checks=cfg.get('nobc', True),
            ),
            name="gated_mix_decode",
        )(A_x, kT, vT, tiles(A_wq, 15), tiles(A_wo, 15), B_w_r,
          tiles(B_w_gate, 4), tiles(B_w_up, 4), tiles(B_w_down, 4), gate_w)
    return fn


def headperm(seq, A, per):
    h = seq[:2 * A]
    t1 = h[:per] + h[per + A:]
    t0 = h[per:per + A]
    return [p for ab in zip(t1, t0) for p in ab] + seq[2 * A:]


P2 = sweep('o4 o2 o3 o2 o3 o1', NC)
DEFAULT['post'] = P2
PRE = DEFAULT['pre']
DEFAULT['pre'] = sweep('q4 q2 q3 q2 q3 q1', NC) + sweep('g4 u2 d4 u2', NC, dict(u=1))


_fn = make()


@jax.jit
def pallas_gated_mix__sliding_block_cached__moe_arch_mod__decode_kernel(
        A_x, A_k_cache, A_v_cache, A_wq, A_wo, B_x, B_w_r, B_w_gate, B_w_up, B_w_down, gate_w):
    return _fn(A_x, A_k_cache, A_v_cache, A_wq, A_wo, B_x, B_w_r, B_w_gate, B_w_up, B_w_down, gate_w)
```

```python
import contextlib
import jax
import jax.numpy as jnp
import jax.experimental.pallas as pl
import jax.experimental.pallas.tpu as pltpu

H, DH, SK, D, F = 32, 192, 32768, 640, 1536
W = min(4096, max(256, SK // 4))
BASE = SK - W
f32 = jnp.float32
bf16 = jnp.bfloat16
NC = dict(q=64, o=64, g=60, u=60, d=60, k=8, v=8)


def sweep(txt, off=None, rev=False):
    split, pos = [], {}
    for t in txt.split():
        k, n = t[0], int(t[1:])
        split.append((k, pos.get(k, 0), n)); pos[k] = pos.get(k, 0) + n
    m = max(NC[k] for k, _, _ in split)
    return [(k, r0, n, ((NC[k] - 1 - c if rev else c) + (off or {}).get(k, 0)) % NC[k])
            for c in range(m) for k, r0, n in split if c < NC[k]]


DEFAULT = dict(
    kv=sweep("k4 k2 " * 4) + sweep("v4 v2 " * 4), L=30, A=11, lag0=4, xat=16, z0=56, dly=0, dly0=0,
    pre=sweep('q4 q2 q3 q2 q3 q1') + sweep('g4 u2 d4 u2', dict(u=1)), post=sweep('o4 o2 o3 o2 o3 o1'),
    nsem=64, scopes=False, A0=99, tb=4,
)


def tiles(w, rows):
    r, c = w.shape
    return w.reshape(r // 8, 8, c // 128, 128).transpose(0, 2, 1, 3).reshape(rows, r * c // 1024 // rows, 8, 128)


def make(**kw):
    cfg = dict(DEFAULT); cfg.update(kw)
    L, A, NSEM, LAG = (cfg[k] for k in ('L', 'A', 'nsem', 'lag0'))
    KV, PRE, POST = cfg['kv'], cfg['pre'], cfg['post']
    SPH, n_pre, n_post = len(KV) // 2, len(PRE) // 2, len(POST) // 2
    assert SPH % NSEM == 0 and L + LAG < min(NSEM, SPH) and len(PRE) % 2 == 0 and len(POST) % 2 == 0

    def scope(name):
        return jax.named_scope(name) if cfg['scopes'] else contextlib.nullcontext()

    def kernel(x_hbm, kT, vT, wq, wo, wr_hbm, wg, wu, wd, gw_hbm, out_ref,
               x_v, wr_v, gw_v, wq_b, k_b, v_b, wo_b, wg_b, wu_b, wd_b,
               x_s, q_s, h_s, o_s, sem1, sem0, sems):
        bufs = dict(q=(wq, wq_b), o=(wo, wo_b), g=(wg, wg_b), u=(wu, wu_b), d=(wd, wd_b), k=(kT, k_b), v=(vT, v_b))

        def copy(q, pos, piece, h):
            k, r0, n, c = piece
            src, dst = bufs[k]
            sem = (sem1, sem0)[q].at[pos % NSEM]
            if k in 'kv':
                rows = pl.ds(r0 * 8, n * 8)
                return pltpu.make_async_copy(src.at[0, h, rows, pl.ds(BASE + c * 512, 512)],
                                             dst.at[rows, pl.ds(c * 512, 512)], sem)
            idx = (pl.ds(r0, n), pl.ds(c * 4, 4))
            return pltpu.make_async_copy(src.at[idx], dst.at[idx], sem)

        def pace(d):
            if d:
                pl.delay(d)

        def step(at, p):
            for q, d, start in ((1, 0, False), (0, LAG, False), (1, LAG + A, True), (0, LAG + L, True)):
                c = at(q, p + d)
                if c is not None:
                    c.start(priority=1 - q) if start else c.wait()

        def column(row):
            return jnp.broadcast_to(row, (128, 128)).T

        def matvec(piece, vec, acc, nt):
            k, r0, n, c = piece
            buf = bufs[k][1]
            for r in range(r0, r0 + n):
                w = buf[r, c * 4:c * 4 + 4].astype(f32)
                for t in range(4):
                    kt, ct = divmod(r * buf.shape[1] + c * 4 + t, nt)
                    part = w[t] * vec[kt * 8:kt * 8 + 8, :]
                    acc[ct] = acc[ct] + part if ct in acc else part

        rowsum = lambda v: jnp.sum(v, axis=0, keepdims=True)

        def pre_at(q, p):
            return copy(q, p, PRE[2 * (p + n_pre) + q] if p < 0 else KV[2 * p + q], 0)

        small = [pltpu.make_async_copy(x_hbm, x_v, sems.at[0]),
                 pltpu.make_async_copy(gw_hbm, gw_v, sems.at[1]),
                 pltpu.make_async_copy(wr_hbm, wr_v, sems.at[2])]
        acc = dict(q={}, g={}, u={}, d={}, o={})
        with scope("zz_pre"):
            for i in range(L + LAG):
                pre_at(0, i - n_pre).start(priority=1)
                if i == 0:
                    for c in small:
                        c.start()
                if i % 3 == 2 and i // 3 < cfg['A0']:
                    pre_at(1, i // 3 - n_pre).start(priority=0)
                    pace(cfg['dly0'])
                    if cfg.get('z0'):
                        wq_b[i // 3, 256 - cfg['z0']:] = jnp.zeros((cfg['z0'], 8, 128), bf16)
            if cfg['A0'] < A:
                small[0].wait()
            for i in range(min(cfg['A0'], (L + LAG) // 3), A):
                pre_at(1, i - n_pre).start(priority=0)
            for i in range(LAG):
                pre_at(0, i - n_pre).wait()
                pre_at(1, A + i - n_pre).start(priority=0)
            done = 0
            q_done = max(j for j, pc in enumerate(PRE) if pc[0] == 'q') // 2 + 1
            tb = cfg['tb']
            gap = max(1, (n_pre - q_done) * tb // 48)
            for i in range(n_pre):
                step(pre_at, i - n_pre)
                if i == cfg['xat']:
                    for c in small[int(cfg['A0'] < A):]:
                        c.wait()
                    xf = x_v[0].astype(f32)
                    gate = jax.nn.sigmoid(jnp.sum(xf * gw_v[...].astype(f32).reshape(1, D), axis=-1, keepdims=True))
                    rsel = jax.nn.sigmoid(jnp.sum(xf * wr_v[...].astype(f32).reshape(1, D), axis=-1, keepdims=True))
                    for j in range(D // 128):
                        x_s[j * 128:(j + 1) * 128, :] = column(xf[:, j * 128:(j + 1) * 128])
                if i > cfg['xat']:
                    upto = min(done + 3, 2 * i + 2)
                    for pc in PRE[done:upto]:
                        if pc[0] != 'd':
                            matvec(pc, x_s, acc[pc[0]], 48 if pc[0] == 'q' else 12)
                    done = upto
                j, rem = divmod(i - q_done, gap)
                if rem == 0 and 0 <= j < 48 // tb:
                    for ct in range(j * tb, (j + 1) * tb):
                        q_s[ct * 128:(ct + 1) * 128, :] = column(rowsum(acc['q'][ct]))
                else:
                    pace(cfg['dly'])

        def head(h, extra=None, last=False):
            def at(q, p):
                if p < SPH:
                    return copy(q, p, KV[2 * p + q], h)
                return copy(q, p, (POST if last else KV)[2 * (p - SPH) + q], h + 1)
            s, o, st, left = {}, {}, {}, {c: 24 for c in range(8)}
            base = pl.multiple_of(h * DH, 8) if not isinstance(h, int) else h * DH
            for p in range(SPH):
                step(at, p)
                slow = False
                for k, r0, n, c in KV[2 * p:2 * p + 2]:
                    if k == 'k':
                        for r in range(r0, r0 + n):
                            part = (k_b[r * 8:r * 8 + 8, c * 512:(c + 1) * 512].astype(f32)
                                    * jnp.tile(q_s[pl.ds(base + r * 8, 8), :], (1, 4)))
                            s[c] = s[c] + part if c in s else part
                        left[c] -= n
                        if left[c] == 0:
                            s[c] = jnp.broadcast_to(rowsum(s[c]), (8, 512)) * DH ** -0.5
                            st['m'] = jnp.maximum(st['m'], s[c]) if 'm' in st else s[c]
                            if not any(left.values()):
                                st['m'] = jnp.max(st['m'], axis=-1, keepdims=True)
                                slow = True
                    else:
                        if ('e', c) not in st:
                            st['e', c] = jnp.exp(s[c] - st['m'])
                            st['l'] = st['l'] + st['e', c] if 'l' in st else st['e', c]
                        for r in range(r0, r0 + n):
                            pv = v_b[r * 8:r * 8 + 8, c * 512:(c + 1) * 512].astype(f32) * st['e', c]
                            part = (pv[:, 0:128] + pv[:, 128:256]) + (pv[:, 256:384] + pv[:, 384:512])
                            o[r] = o[r] + part if r in o else part
                if extra is not None:
                    slow = extra(p) or slow
                if not slow and p < SPH - 1:
                    pace(cfg['dly'])
            inv = 1.0 / jnp.sum(st['l'], axis=-1, keepdims=True)
            for r in range(DH // 8):
                o_s[pl.ds(base + r * 8, 8), :] = jnp.broadcast_to(jnp.sum(o[r], axis=-1, keepdims=True) * inv, (8, 128))

        late = [pc for pc in PRE if pc[0] == 'd']

        def ffn(p):
            if p in (4, 10, 16):
                for ct in range(4 * (p // 6), 4 * (p // 6) + 4):
                    h_s[ct * 128:(ct + 1) * 128, :] = column(jax.nn.silu(rowsum(acc['g'][ct])) * rowsum(acc['u'][ct]))
                return True
            per = -(-len(late) // (SPH - 17))
            for pc in late[max(0, p - 17) * per:max(0, p - 16) * per]:
                matvec(pc, h_s, acc['d'], 5)

        with scope("zz_loop"):
            jax.lax.fori_loop(0, H - 1, lambda h, _: head(h), None)
        with scope("zz_h31"):
            head(H - 1, ffn, last=True)

        def post_at(q, p):
            return copy(q, p, POST[2 * p + q], None) if p < n_post else None

        def side():
            y = rowsum(jnp.concatenate([acc['d'][c] for c in range(5)], axis=1))
            return (1.0 - gate) * (xf + (xf * 0.0 + y * rsel))

        d_done = max([j // 2 for j, pc in enumerate(POST) if pc[0] == 'd'], default=0)
        with scope("zz_post"):
            n_main = n_post - LAG - A
            for p in range(n_post):
                if p < n_main:
                    step(post_at, p)
                for q in range(2):
                    if p >= n_main + (0 if q else LAG):
                        post_at(q, p).wait()
                    pc = POST[2 * p + q]
                    matvec(pc, o_s if pc[0] == 'o' else h_s, acc[pc[0]], 5)
                if p == d_done:
                    b = side()
                if p + 1 < n_main:
                    pace(cfg['dly'])
            a = rowsum(jnp.concatenate([acc['o'][c] for c in range(5)], axis=1))
            out_ref[0] = (gate * a + b).astype(bf16)

    def fn(A_x, A_k_cache, A_v_cache, A_wq, A_wo, B_x, B_w_r, B_w_gate, B_w_up, B_w_down, gate_w):
        del B_x
        any_spec = pl.BlockSpec(memory_space=pl.ANY)
        vmem = pltpu.VMEM
        big, ffn = vmem((15, 256, 8, 128), bf16), vmem((4, 240, 8, 128), bf16)
        return pl.pallas_call(
            kernel,
            out_shape=jax.ShapeDtypeStruct((1, 1, D), bf16),
            in_specs=[any_spec] * 10,
            out_specs=pl.BlockSpec(memory_space=pltpu.VMEM),
            scratch_shapes=[
                vmem((1, 1, D), bf16), vmem((D,), bf16), vmem((D,), bf16),
                big, vmem((DH, W), bf16), vmem((DH, W), bf16), big, ffn, ffn, ffn,
                vmem((D, 128), f32), vmem((H * DH, 128), f32), vmem((F, 128), f32), vmem((H * DH, 128), f32),
                pltpu.SemaphoreType.DMA((NSEM,)), pltpu.SemaphoreType.DMA((NSEM,)),
                pltpu.SemaphoreType.DMA((3,)),
            ],
            compiler_params=pltpu.CompilerParams(
                vmem_limit_bytes=64 * 1024 * 1024,
                disable_semaphore_checks=True, disable_bounds_checks=cfg.get('nobc', True),
            ),
            name="gated_mix_decode",
        )(A_x, jnp.swapaxes(A_k_cache, 2, 3), jnp.swapaxes(A_v_cache, 2, 3), tiles(A_wq, 15), tiles(A_wo, 15), B_w_r,
          tiles(B_w_gate, 4), tiles(B_w_up, 4), tiles(B_w_down, 4), gate_w)
    return fn

O3 = sweep('o3 ' * 5)
Q3 = sweep('q3 ' * 5)
Q4 = sweep('q4 q2 q3 q2 q3 q1')
GUD = sweep('g4 u2 d4 u2', dict(u=1))


_fn = make()


@jax.jit
def pallas_gated_mix__sliding_block_cached__moe_arch_mod__decode_kernel(
        A_x, A_k_cache, A_v_cache, A_wq, A_wo, B_x, B_w_r, B_w_gate, B_w_up, B_w_down, gate_w):
    return _fn(A_x, A_k_cache, A_v_cache, A_wq, A_wo, B_x, B_w_r, B_w_gate, B_w_up, B_w_down, gate_w)
```

```python
import contextlib
import jax
import jax.numpy as jnp
import jax.experimental.pallas as pl
import jax.experimental.pallas.tpu as pltpu

H, DH, SK, D, F = 32, 192, 32768, 640, 1536
W = min(4096, max(256, SK // 4))
BASE = SK - W
f32 = jnp.float32
bf16 = jnp.bfloat16
NC = dict(q=64, o=64, g=60, u=60, d=60, k=8, v=8)


def sweep(txt, off=None, rev=False, FR=4):
    NC = dict(q=64, o=64, g=240 // FR, u=240 // FR, d=240 // FR, k=8, v=8)
    split, pos = [], {}
    for t in txt.split():
        k, n = t[0], int(t[1:])
        split.append((k, pos.get(k, 0), n)); pos[k] = pos.get(k, 0) + n
    m = max(NC[k] for k, _, _ in split)
    return [(k, r0, n, ((NC[k] - 1 - c if rev else c) + (off or {}).get(k, 0)) % NC[k])
            for c in range(m) for k, r0, n in split if c < NC[k]]


DEFAULT = dict(
    kv=sweep("k4 k2 " * 4) + sweep("v4 v2 " * 4), L=30, A=11, lag0=4, xat=16, z0=56, dly=0, dly0=0,
    pre=sweep('q4 q2 q3 q2 q3 q1') + sweep('g4 u2 d4 u2', dict(u=1)), post=sweep('o4 o2 o3 o2 o3 o1'),
    nsem=64, scopes=False, A0=99, tb=4,
)


def tiles(w, rows):
    r, c = w.shape
    return w.reshape(r // 8, 8, c // 128, 128).transpose(0, 2, 1, 3).reshape(rows, r * c // 1024 // rows, 8, 128)


def make(**kw):
    cfg = dict(DEFAULT); cfg.update(kw)
    L, A, NSEM, LAG = (cfg[k] for k in ('L', 'A', 'nsem', 'lag0'))
    ST = cfg.get('ST', 1)
    FR = cfg.get('FR', 4)
    KV, PRE, POST = cfg['kv'], cfg['pre'], cfg['post']
    SPH, n_pre, n_post = len(KV) // 2, len(PRE) // 2, len(POST) // 2
    assert SPH % NSEM == 0 and L + LAG < min(NSEM, SPH) and len(PRE) % 2 == 0 and len(POST) % 2 == 0

    def scope(name):
        return jax.named_scope(name) if cfg['scopes'] else contextlib.nullcontext()

    def kernel(x_hbm, kT, vT, wq, wo, wr_hbm, wg, wu, wd, gw_hbm, out_ref,
               x_v, wr_v, gw_v, wq_b, k_b, v_b, wo_b, wg_b, wu_b, wd_b,
               x_s, q_s, h_s, o_s, sem1, sem0, sems):
        bufs = dict(q=(wq, wq_b), o=(wo, wo_b), g=(wg, wg_b), u=(wu, wu_b), d=(wd, wd_b), k=(kT, k_b), v=(vT, v_b))

        def copy(q, pos, piece, h):
            k, r0, n, c = piece
            src, dst = bufs[k]
            sem = (sem1, sem0)[q].at[pos % NSEM]
            if k in 'kv':
                rows = (pl.ds(r0 // ST, n), pl.ds((r0 % ST) * 8, 8))
                return pltpu.make_async_copy(src.at[h, *rows, pl.ds(BASE + c * 512, 512 * ST)],
                                             dst.at[*rows, pl.ds(c * 512, 512 * ST)], sem)
            idx = (pl.ds(r0, n), pl.ds(c * 4, 4))
            return pltpu.make_async_copy(src.at[idx], dst.at[idx], sem)

        def pace(d):
            if d:
                pl.delay(d)

        def step(at, p):
            for q, d, start in ((1, 0, False), (0, LAG, False), (1, LAG + A, True), (0, LAG + L, True)):
                c = at(q, p + d)
                if c is not None:
                    c.start(priority=1 - q) if start else c.wait()

        def column(row):
            return jnp.broadcast_to(row, (128, 128)).T

        def matvec(piece, vec, acc, nt):
            k, r0, n, c = piece
            buf = bufs[k][1]
            for r in range(r0, r0 + n):
                w = buf[r, c * 4:c * 4 + 4].astype(f32)
                for t in range(4):
                    kt, ct = divmod(r * buf.shape[1] + c * 4 + t, nt)
                    part = w[t] * vec[kt * 8:kt * 8 + 8, :]
                    acc[ct] = acc[ct] + part if ct in acc else part

        rowsum = lambda v: jnp.sum(v, axis=0, keepdims=True)

        def pre_at(q, p):
            return copy(q, p, PRE[2 * (p + n_pre) + q] if p < 0 else KV[2 * p + q], 0)

        small = [pltpu.make_async_copy(x_hbm, x_v, sems.at[0]),
                 pltpu.make_async_copy(gw_hbm, gw_v, sems.at[1]),
                 pltpu.make_async_copy(wr_hbm, wr_v, sems.at[2])]
        acc = dict(q={}, g={}, u={}, d={}, o={})
        with scope("zz_pre"):
            for i in range(L + LAG):
                pre_at(0, i - n_pre).start(priority=1)
                if i == 0:
                    for c in small:
                        c.start()
                if i % 3 == 2 and i // 3 < cfg['A0']:
                    pre_at(1, i // 3 - n_pre).start(priority=0)
                    pace(cfg['dly0'])
                    if cfg.get('z0'):
                        wq_b[i // 3, 256 - cfg['z0']:] = jnp.zeros((cfg['z0'], 8, 128), bf16)
            if cfg['A0'] < A:
                small[0].wait()
            for i in range(min(cfg['A0'], (L + LAG) // 3), A):
                pre_at(1, i - n_pre).start(priority=0)
            for i in range(LAG):
                pre_at(0, i - n_pre).wait()
                pre_at(1, A + i - n_pre).start(priority=0)
            done = 0
            q_done = max(j for j, pc in enumerate(PRE) if pc[0] == 'q') // 2 + 1
            tb = cfg['tb']
            gap = max(1, (n_pre - q_done) * tb // 48)
            for i in range(n_pre):
                with (scope('zz_mark') if i in (0, q_done) else contextlib.nullcontext()):
                    step(pre_at, i - n_pre)
                if i == cfg['xat']:
                    for c in small[int(cfg['A0'] < A):]:
                        c.wait()
                    xf = x_v[0].astype(f32)
                    gate = jax.nn.sigmoid(jnp.sum(xf * gw_v[...].astype(f32).reshape(1, D), axis=-1, keepdims=True))
                    rsel = jax.nn.sigmoid(jnp.sum(xf * wr_v[...].astype(f32).reshape(1, D), axis=-1, keepdims=True))
                    for j in range(D // 128):
                        x_s[j * 128:(j + 1) * 128, :] = column(xf[:, j * 128:(j + 1) * 128])
                if i > cfg['xat']:
                    upto = min(done + 3, 2 * i + 2)
                    for pc in PRE[done:upto]:
                        if pc[0] != 'd':
                            matvec(pc, x_s, acc[pc[0]], 48 if pc[0] == 'q' else 12)
                    done = upto
                j, rem = divmod(i - q_done, gap)
                if rem == 0 and 0 <= j < 48 // tb:
                    for ct in range(j * tb, (j + 1) * tb):
                        q_s[ct * 128:(ct + 1) * 128, :] = column(rowsum(acc['q'][ct]))
                else:
                    pace(cfg['dly'])

        def head(h, extra=None, last=False):
            def at(q, p):
                if p < SPH:
                    return copy(q, p, KV[2 * p + q], h)
                return copy(q, p, (POST if last else KV)[2 * (p - SPH) + q], h + 1)
            s, o, st, left = {}, {}, {}, {c: 24 for c in range(8)}
            base = pl.multiple_of(h * DH, 8) if not isinstance(h, int) else h * DH
            for p in range(SPH):
                step(at, p)
                slow = False
                for k, r0, n, c in [(k, r0, n, c + j) for k, r0, n, c in KV[2 * p:2 * p + 2] for j in range(ST)]:
                    if k == 'k':
                        for r in range(r0, r0 + n * ST, ST):
                            part = (k_b[r // ST, (r % ST) * 8:(r % ST) * 8 + 8, c * 512:(c + 1) * 512].astype(f32)
                                    * jnp.tile(q_s[pl.ds(base + r * 8, 8), :], (1, 4)))
                            s[c] = s[c] + part if c in s else part
                        left[c] -= n
                        if left[c] == 0:
                            s[c] = jnp.broadcast_to(rowsum(s[c]), (8, 512)) * DH ** -0.5
                            st['m'] = jnp.maximum(st['m'], s[c]) if 'm' in st else s[c]
                            if not any(left.values()):
                                st['m'] = jnp.max(st['m'], axis=-1, keepdims=True)
                                slow = True
                    else:
                        if ('e', c) not in st:
                            st['e', c] = jnp.exp(s[c] - st['m'])
                            st['l'] = st['l'] + st['e', c] if 'l' in st else st['e', c]
                        for r in range(r0, r0 + n * ST, ST):
                            pv = v_b[r // ST, (r % ST) * 8:(r % ST) * 8 + 8, c * 512:(c + 1) * 512].astype(f32) * st['e', c]
                            part = (pv[:, 0:128] + pv[:, 128:256]) + (pv[:, 256:384] + pv[:, 384:512])
                            o[r] = o[r] + part if r in o else part
                if extra is not None:
                    slow = extra(p) or slow
                if not slow and p < SPH - 1 and not last:
                    pace(cfg.get('dk', 0) if k == 'k' else cfg.get('dv', 0))
            inv = 1.0 / jnp.sum(st['l'], axis=-1, keepdims=True)
            for r in range(DH // 8):
                o_s[pl.ds(base + r * 8, 8), :] = jnp.broadcast_to(jnp.sum(o[r], axis=-1, keepdims=True) * inv, (8, 128))

        late = [pc for pc in PRE if pc[0] == 'd']

        def ffn(p):
            if p in (4, 10, 16):
                for ct in range(4 * (p // 6), 4 * (p // 6) + 4):
                    h_s[ct * 128:(ct + 1) * 128, :] = column(jax.nn.silu(rowsum(acc['g'][ct])) * rowsum(acc['u'][ct]))
                return True
            per = -(-len(late) // (SPH - 17))
            for pc in late[max(0, p - 17) * per:max(0, p - 16) * per]:
                matvec(pc, h_s, acc['d'], 5)

        with scope("zz_loop"):
            jax.lax.fori_loop(0, H - 1, lambda h, _: head(h), None)
        with scope("zz_h31"):
            head(H - 1, ffn, last=True)

        def post_at(q, p):
            return copy(q, p, POST[2 * p + q], None) if p < n_post else None

        def side():
            y = rowsum(jnp.concatenate([acc['d'][c] for c in range(5)], axis=1))
            return (1.0 - gate) * (xf + (xf * 0.0 + y * rsel))

        d_done = max([j // 2 for j, pc in enumerate(POST) if pc[0] == 'd'], default=0)
        with scope("zz_post"):
            n_main = n_post - LAG - A
            for p in range(n_post):
                if p < n_main:
                    step(post_at, p)
                for q in range(2):
                    if p >= n_main + (0 if q else LAG):
                        post_at(q, p).wait()
                    pc = POST[2 * p + q]
                    matvec(pc, o_s if pc[0] == 'o' else h_s, acc[pc[0]], 5)
                if p == d_done:
                    b = side()
                if p + 1 < n_main:
                    pace(cfg['dly'])
            a = rowsum(jnp.concatenate([acc['o'][c] for c in range(5)], axis=1))
            out_ref[0] = (gate * a + b).astype(bf16)

    def fn(A_x, A_k_cache, A_v_cache, A_wq, A_wo, B_x, B_w_r, B_w_gate, B_w_up, B_w_down, gate_w):
        del B_x
        any_spec = pl.BlockSpec(memory_space=pl.ANY)
        vmem = pltpu.VMEM
        big, ffn = vmem((15, 256, 8, 128), bf16), vmem((FR, 960 // FR, 8, 128), bf16)
        return pl.pallas_call(
            kernel,
            out_shape=jax.ShapeDtypeStruct((1, 1, D), bf16),
            in_specs=[any_spec] * 10,
            out_specs=pl.BlockSpec(memory_space=pltpu.VMEM),
            scratch_shapes=[
                vmem((1, 1, D), bf16), vmem((D,), bf16), vmem((D,), bf16),
                big, vmem((24 // ST, 8 * ST, W), bf16), vmem((24 // ST, 8 * ST, W), bf16), big, ffn, ffn, ffn,
                vmem((D, 128), f32), vmem((H * DH, 128), f32), vmem((F, 128), f32), vmem((H * DH, 128), f32),
                pltpu.SemaphoreType.DMA((NSEM,)), pltpu.SemaphoreType.DMA((NSEM,)),
                pltpu.SemaphoreType.DMA((3,)),
            ],
            compiler_params=pltpu.CompilerParams(
                vmem_limit_bytes=64 * 1024 * 1024,
                disable_semaphore_checks=True, disable_bounds_checks=cfg.get('nobc', True),
            ),
            name="gated_mix_decode",
        )(A_x, jnp.swapaxes(A_k_cache, 2, 3).reshape(H, 24 // ST, 8 * ST, SK), jnp.swapaxes(A_v_cache, 2, 3).reshape(H, 24 // ST, 8 * ST, SK), tiles(A_wq, 15), tiles(A_wo, 15), B_w_r,
          tiles(B_w_gate, FR), tiles(B_w_up, FR), tiles(B_w_down, FR), gate_w)
    return fn

O3 = sweep('o3 ' * 5)
Q3 = sweep('q3 ' * 5)
Q4 = sweep('q4 q2 q3 q2 q3 q1')
GUD = sweep('g4 u2 d4 u2', dict(u=1))


def segs(ST, k, v=None):
    out = []
    for a, txt in (('k', k), ('v', v or k)):
        for t in txt.split():
            r, c = map(int, t.split('.'))
            out += [(a, r, 4 // ST, c), (a, r + 4, 2 // ST, c)]
    return dict(ST=ST, kv=out)


K1 = "12.0 18.0 0.0 6.0 12.3 18.3 0.3 6.3 12.2 18.2 0.2 6.2 12.1 18.1 0.1 6.1 12.4 18.4 0.4 6.4 12.7 18.7 0.7 6.7 12.6 18.6 0.6 6.6 12.5 18.5 0.5 6.5"
K2 = "6.0 12.0 18.0 0.0 6.2 12.2 18.2 0.2 7.0 13.0 19.0 1.0 7.2 13.2 19.2 1.2 6.4 12.4 18.4 0.4 6.6 12.6 18.6 0.6 7.4 13.4 19.4 1.4 7.6 13.6 19.6 1.6"
V1 = "6.0 12.0 18.0 0.0 6.1 12.1 18.1 0.1 6.2 12.2 18.2 0.2 6.5 12.5 18.5 0.5 6.4 12.4 18.4 0.4 6.3 12.3 18.3 0.3 6.6 12.6 18.6 0.6 6.7 12.7 18.7 0.7"
V2 = "7.2 13.2 19.2 1.2 7.4 13.4 19.4 1.4 6.0 12.0 18.0 0.0 6.2 12.2 18.2 0.2 6.4 12.4 18.4 0.4 7.0 13.0 19.0 1.0 6.6 12.6 18.6 0.6 7.6 13.6 19.6 1.6"


def runs(k, v):
    out = []
    for a, g in (('k', k), ('v', v)):
        for res, c, rot, rev in g:
            seg = [((rot + 3 * i) % 12) for i in range(4)]
            for s in (seg[::-1] if rev else seg):
                out += [(a, 2 * s + res, 2, c), (a, 2 * ((s + 2) % 12) + res, 1, c)]
    return dict(ST=2, kv=out, A=12, L=32)


KA = [(0, 2, 3, 1), (0, 0, 3, 1), (1, 0, 6, 0), (1, 2, 3, 0), (0, 6, 3, 0), (0, 4, 0, 0), (1, 4, 10, 0), (1, 6, 0, 0)]
KB = [(0, 2, 3, 0), (0, 0, 3, 0), (1, 0, 6, 0), (1, 2, 3, 0), (0, 6, 3, 0), (0, 4, 0, 0), (1, 4, 9, 0), (1, 6, 0, 0)]
KC = [(0, 2, 3, 0), (0, 0, 3, 0), (1, 0, 3, 0), (1, 2, 3, 0), (0, 6, 3, 0), (0, 4, 3, 0), (1, 4, 3, 0), (1, 6, 3, 0)]
VA = [(1, 2, 3, 1), (1, 4, 3, 0), (0, 0, 0, 1), (0, 2, 0, 0), (0, 4, 7, 1), (1, 0, 3, 0), (0, 6, 0, 0), (1, 6, 3, 0)]
VB = [(1, 2, 3, 0), (1, 4, 3, 0), (0, 0, 0, 0), (0, 2, 0, 0), (0, 4, 0, 0), (1, 0, 3, 0), (0, 6, 0, 0), (1, 6, 3, 0)]
GG = lambda s: [(int(t[0]), int(t[1]), 0, 0) for t in s.split()]
DEFAULT.update(runs(GG("02 00 10 12 06 04 14 16"), GG("00 02 04 10 12 14 06 16")))


_fn = make()


@jax.jit
def pallas_gated_mix__sliding_block_cached__moe_arch_mod__decode_kernel(
        A_x, A_k_cache, A_v_cache, A_wq, A_wo, B_x, B_w_r, B_w_gate, B_w_up, B_w_down, gate_w):
    return _fn(A_x, A_k_cache, A_v_cache, A_wq, A_wo, B_x, B_w_r, B_w_gate, B_w_up, B_w_down, gate_w)
```

```python
import jax
import jax.numpy as jnp
import jax.experimental.pallas as pl
import jax.experimental.pallas.tpu as pltpu

H, DH, SK, D, F = 32, 192, 32768, 640, 1536
W = min(4096, max(256, SK // 4))
BASE = SK - W

LOOK1, LOOK0 = 32, 12
LAG = 4
NSEM = 64
X_STEP = 16

f32 = jnp.float32
bf16 = jnp.bfloat16

REGIONS = dict(q=(15, 256), o=(15, 256), g=(4, 240), u=(4, 240), d=(4, 240))
COL_TILES = dict(q=H * DH // 128, o=D // 128, g=F // 128, u=F // 128, d=D // 128)
TW = 4
KC = 1024


def _sweep(*split):
    return [(name, r0, n, t) for t in range(0, REGIONS[split[0][0]][1], TW) for name, r0, n in split]


def _kv_sweep(name, runs):
    return [(name, g + dg, n, (half, col * KC))
            for half, col in runs for g in range(0, DH // 16, 3) for dg, n in ((0, 2), (2, 1))]


_SPLIT15 = ((0, 4), (4, 2), (6, 3), (9, 2), (11, 3), (14, 1))
PRE = (_sweep(*[('q', r0, n) for r0, n in _SPLIT15])
       + _sweep(('g', 0, 4), ('u', 0, 2), ('d', 0, 4), ('u', 2, 2)))
HEAD = (_kv_sweep('k', ((0, 1), (0, 0), (1, 0), (1, 1), (0, 3), (0, 2), (1, 2), (1, 3)))
        + _kv_sweep('v', ((0, 0), (0, 1), (0, 2), (1, 0), (1, 1), (1, 2), (0, 3), (1, 3))))
POST = _sweep(*[('o', r0, n) for r0, n in _SPLIT15])
N_PRE, N_HEAD, N_POST = len(PRE) // 2, len(HEAD) // 2, len(POST) // 2
assert N_HEAD % NSEM == 0 and LOOK0 <= LOOK1 and LAG + LOOK1 < min(NSEM, N_HEAD)


def _rowsum(v):
    return jnp.sum(v, axis=0, keepdims=True)


def _column(row):
    return jnp.broadcast_to(row, (128, 128)).T


def _accumulate(acc, key, part):
    acc[key] = acc[key] + part if key in acc else part


def _kernel(x_hbm, kT, vT, wq, wo, wr_hbm, wg, wu, wd, gw_hbm, out_ref,
            x_v, wr_v, gw_v, k_b, v_b, wq_b, wo_b, wg_b, wu_b, wd_b,
            x_s, q_s, h_s, o_s, sem1, sem0, sem_small):
    bufs = dict(k=(kT, k_b), v=(vT, v_b), q=(wq, wq_b), o=(wo, wo_b),
                g=(wg, wg_b), u=(wu, wu_b), d=(wd, wd_b))

    def copy(odd, pos, piece, h=None):
        name, r0, n, col = piece
        src, dst = bufs[name]
        sem = (sem1, sem0)[odd].at[pos % NSEM]
        if name in 'kv':
            half, c = col
            g, rows = pl.ds(r0, n), pl.ds(half * 8, 8)
            return pltpu.make_async_copy(src.at[h, g, rows, pl.ds(BASE + c, KC)],
                                         dst.at[g, rows, pl.ds(c, KC)], sem)
        idx = (pl.ds(r0, n), pl.ds(col, TW))
        return pltpu.make_async_copy(src.at[idx], dst.at[idx], sem)

    def step(at, p):
        at(1, p).wait()
        at(0, p + LAG).wait()
        at(1, p + LAG + LOOK0).start(priority=0)
        nxt = at(0, p + LAG + LOOK1)
        if nxt is not None:
            nxt.start(priority=1)

    acc = {name: {} for name in REGIONS}

    def matvec(piece, vec):
        name, r0, n, t0 = piece
        for r in range(r0, r0 + n):
            w = bufs[name][1][r, t0:t0 + TW].astype(f32)
            for t in range(TW):
                kt, ct = divmod(r * REGIONS[name][1] + t0 + t, COL_TILES[name])
                _accumulate(acc[name], ct, w[t] * vec[kt * 8:kt * 8 + 8, :])

    def pre_at(odd, p):
        return copy(odd, p, PRE[2 * (p + N_PRE) + odd] if p < 0 else HEAD[2 * p + odd], 0)

    small = [pltpu.make_async_copy(x_hbm, x_v, sem_small.at[0]),
             pltpu.make_async_copy(gw_hbm, gw_v, sem_small.at[1]),
             pltpu.make_async_copy(wr_hbm, wr_v, sem_small.at[2])]
    per = (LAG + LOOK1) // LOOK0
    assert per * LOOK0 == LAG + LOOK1
    for i in range(LOOK0):
        for j in range(i * per, (i + 1) * per):
            pre_at(0, j - N_PRE).start(priority=1)
        pre_at(1, i - N_PRE).start(priority=0)
        wq_b[i, 200:] = jnp.zeros((56, 8, 128), bf16)
    for c in small:
        c.start()
    for i in range(LAG):
        pre_at(0, i - N_PRE).wait()
        pre_at(1, LOOK0 + i - N_PRE).start(priority=0)

    q_done = sum(piece[0] == 'q' for piece in PRE) // 2
    used = 0
    for i in range(N_PRE):
        step(pre_at, i - N_PRE)
        if i == X_STEP:
            for c in small:
                c.wait()
            x = x_v[0].astype(f32)
            gate = jax.nn.sigmoid(jnp.sum(x * gw_v[...].astype(f32).reshape(1, D), axis=-1, keepdims=True))
            rsel = jax.nn.sigmoid(jnp.sum(x * wr_v[...].astype(f32).reshape(1, D), axis=-1, keepdims=True))
            for j in range(0, D, 128):
                x_s[j:j + 128, :] = _column(x[:, j:j + 128])
        elif i > X_STEP:
            upto = min(used + 3, 2 * i + 2)
            for piece in PRE[used:upto]:
                if piece[0] != 'd':
                    matvec(piece, x_s)
            used = upto
        if i >= q_done and (i - q_done) % 10 == 0:
            assert used >= 2 * q_done
            for ct in range((i - q_done) // 10 * 4, (i - q_done) // 10 * 4 + 4):
                q_s[ct * 128:(ct + 1) * 128, :] = _column(_rowsum(acc['q'].pop(ct)))
    assert used == len(PRE) and not acc['q']

    def head(h, following, extra=None):
        def at(odd, p):
            if p < N_HEAD:
                return copy(odd, p, HEAD[2 * p + odd], h)
            return copy(odd, p, following[2 * (p - N_HEAD) + odd], h + 1)

        s, e, o, stat = {}, {}, {}, {}
        missing = {c: DH // 8 for c in range(0, W, KC)}
        for p in range(N_HEAD):
            step(at, p)
            for name, g0, n, (half, c) in HEAD[2 * p:2 * p + 2]:
                rows, cols = slice(half * 8, half * 8 + 8), slice(c, c + KC)
                if name == 'k':
                    for g in range(g0, g0 + n):
                        r0 = h * DH + g * 16 + half * 8
                        q = q_s[pl.ds(r0 if isinstance(r0, int) else pl.multiple_of(r0, 8), 8), :]
                        _accumulate(s, c, k_b[g, rows, cols].astype(f32) * jnp.tile(q, (1, KC // 128)))
                    missing[c] -= n
                    if missing[c] == 0:
                        s[c] = jnp.broadcast_to(_rowsum(s[c]), (8, KC)) * DH ** -0.5
                        for j in range(0, KC, 128):
                            tile = s[c][:, j:j + 128]
                            stat['max'] = jnp.maximum(stat['max'], tile) if 'max' in stat else tile
                        if not any(missing.values()):
                            row_max = jnp.max(stat['max'], axis=-1, keepdims=True)
                else:
                    if c not in e:
                        e[c] = jnp.exp(s[c] - row_max)
                        for j in range(0, KC, 128):
                            _accumulate(stat, 'sum', e[c][:, j:j + 128])
                    for g in range(g0, g0 + n):
                        pv = v_b[g, rows, cols].astype(f32) * e[c]
                        parts = [pv[:, j:j + 128] for j in range(0, KC, 128)]
                        while len(parts) > 1:
                            parts = [a + b for a, b in zip(parts[::2], parts[1::2])]
                        _accumulate(o, g * 16 + half * 8, parts[0])
            if extra is not None:
                extra(p)
        inv = 1.0 / jnp.sum(stat['sum'], axis=-1, keepdims=True)
        for r in range(0, DH, 8):
            r0 = h * DH + r
            o_s[pl.ds(r0 if isinstance(r0, int) else pl.multiple_of(r0, 8), 8), :] = jnp.broadcast_to(
                jnp.sum(o[r], axis=-1, keepdims=True) * inv, (8, 128))

    down = [piece for piece in PRE if piece[0] == 'd']

    def ffn(p):
        if p in (4, 10, 16):
            for ct in range(p // 6 * 4, p // 6 * 4 + 4):
                hidden = jax.nn.silu(_rowsum(acc['g'][ct])) * _rowsum(acc['u'][ct])
                h_s[ct * 128:(ct + 1) * 128, :] = _column(hidden)
        elif p > 16:
            for piece in down[(p - 17) * 2:(p - 16) * 2]:
                matvec(piece, h_s)

    assert 17 + len(down) // 2 <= N_HEAD
    jax.lax.fori_loop(0, H - 1, lambda h, _: head(h, HEAD), None)
    head(H - 1, POST, ffn)

    def post_at(odd, p):
        return copy(odd, p, POST[2 * p + odd]) if p < N_POST else None

    y = _rowsum(jnp.concatenate([acc['d'][ct] for ct in range(D // 128)], axis=1))
    b = (1.0 - gate) * (x + (x * 0.0 + y * rsel))
    n_issue = N_POST - LAG - LOOK0
    for p in range(N_POST):
        if p < n_issue:
            step(post_at, p)
        for odd in (1, 0):
            if p >= n_issue + (0 if odd else LAG):
                post_at(odd, p).wait()
            matvec(POST[2 * p + odd], o_s)
    a = _rowsum(jnp.concatenate([acc['o'][ct] for ct in range(D // 128)], axis=1))
    out_ref[0] = (gate * a + b).astype(bf16)


def _tiles(w, name):
    r, c = w.shape
    return w.reshape(r // 8, 8, c // 128, 128).transpose(0, 2, 1, 3).reshape(*REGIONS[name], 8, 128)


@jax.jit
def pallas_gated_mix__sliding_block_cached__moe_arch_mod__decode_kernel(
        A_x, A_k_cache, A_v_cache, A_wq, A_wo, B_x, B_w_r, B_w_gate, B_w_up, B_w_down, gate_w):
    del B_x
    kT = jnp.swapaxes(A_k_cache, 2, 3).reshape(H, DH // 16, 16, SK)
    vT = jnp.swapaxes(A_v_cache, 2, 3).reshape(H, DH // 16, 16, SK)
    vmem = pltpu.VMEM
    return pl.pallas_call(
        _kernel,
        out_shape=jax.ShapeDtypeStruct((1, 1, D), bf16),
        in_specs=[pl.BlockSpec(memory_space=pl.ANY)] * 10,
        out_specs=pl.BlockSpec(memory_space=pltpu.VMEM),
        scratch_shapes=[
            vmem((1, 1, D), bf16), vmem((D,), bf16), vmem((D,), bf16),
            vmem((DH // 16, 16, W), bf16), vmem((DH // 16, 16, W), bf16),
            *[vmem((*REGIONS[name], 8, 128), bf16) for name in 'qogud'],
            vmem((D, 128), f32), vmem((H * DH, 128), f32), vmem((F, 128), f32), vmem((H * DH, 128), f32),
            pltpu.SemaphoreType.DMA((NSEM,)), pltpu.SemaphoreType.DMA((NSEM,)),
            pltpu.SemaphoreType.DMA((3,)),
        ],
        compiler_params=pltpu.CompilerParams(
            vmem_limit_bytes=64 * 1024 * 1024,
            disable_semaphore_checks=True,
            disable_bounds_checks=True,
        ),
        name="gated_mix_decode",
    )(A_x, kT, vT, _tiles(A_wq, 'q'), _tiles(A_wo, 'o'), B_w_r,
      _tiles(B_w_gate, 'g'), _tiles(B_w_up, 'u'), _tiles(B_w_down, 'd'), gate_w)
```

```python
import jax
import jax.numpy as jnp
import jax.experimental.pallas as pl
import jax.experimental.pallas.tpu as pltpu

H, DH, SK, D, F = 32, 192, 32768, 640, 1536
W = min(4096, max(256, SK // 4))
BASE = SK - W

LOOK1, LOOK0 = 32, 12
LAG = 4
NSEM = 64
X_STEP = 16

f32 = jnp.float32
bf16 = jnp.bfloat16

REGIONS = dict(q=(15, 256), o=(15, 256), g=(4, 240), u=(4, 240), d=(4, 240))
COL_TILES = dict(q=H * DH // 128, o=D // 128, g=F // 128, u=F // 128, d=D // 128)
TW = 4
KC = 1024


def _sweep(*split):
    return [(name, r0, n, (t, TW)) for t in range(0, REGIONS[split[0][0]][1], TW) for name, r0, n in split]


def _kv_sweep(name, runs):
    return [(name, g + dg, n, (half, col * KC))
            for half, col in runs for g in range(0, DH // 16, 3) for dg, n in ((0, 2), (2, 1))]


_SPLIT15 = ((0, 4), (4, 2), (6, 3), (9, 2), (11, 3), (14, 1))
PRE = (_sweep(*[('q', r0, n) for r0, n in _SPLIT15])
       + _sweep(('g', 0, 4), ('u', 0, 2), ('d', 0, 4), ('u', 2, 2)))
HEAD = (_kv_sweep('k', ((0, 1), (0, 0), (1, 0), (1, 1), (0, 3), (0, 2), (1, 2), (1, 3)))
        + _kv_sweep('v', ((0, 0), (0, 1), (0, 2), (1, 0), (1, 1), (1, 2), (0, 3), (1, 3))))
POST = ([p for p in _sweep(*[('o', r0, n) for r0, n in _SPLIT15]) if p[1] < 11 or p[3][0] < 208]
        + [('o', r, 1, (t, 12)) for r in range(11, 15) for t in range(208, 256, 12)])
N_PRE, N_HEAD, N_POST = len(PRE) // 2, len(HEAD) // 2, len(POST) // 2
assert N_HEAD % NSEM == 0 and LOOK0 <= LOOK1 and LAG + LOOK1 < min(NSEM, N_HEAD)


def _rowsum(v):
    return jnp.sum(v, axis=0, keepdims=True)


def _column(row):
    return jnp.broadcast_to(row, (128, 128)).T


def _accumulate(acc, key, part):
    acc[key] = acc[key] + part if key in acc else part


def _kernel(x_hbm, kT, vT, wq, wo, wr_hbm, wg, wu, wd, gw_hbm, out_ref,
            x_v, wr_v, gw_v, k_b, v_b, wq_b, wo_b, wg_b, wu_b, wd_b,
            x_s, q_s, h_s, o_s, sem1, sem0, sem_small):
    bufs = dict(k=(kT, k_b), v=(vT, v_b), q=(wq, wq_b), o=(wo, wo_b),
                g=(wg, wg_b), u=(wu, wu_b), d=(wd, wd_b))

    def copy(odd, pos, piece, h=None):
        name, r0, n, col = piece
        src, dst = bufs[name]
        sem = (sem1, sem0)[odd].at[pos % NSEM]
        if name in 'kv':
            half, c = col
            g, rows = pl.ds(r0, n), pl.ds(half * 8, 8)
            return pltpu.make_async_copy(src.at[h, g, rows, pl.ds(BASE + c, KC)],
                                         dst.at[g, rows, pl.ds(c, KC)], sem)
        idx = (pl.ds(r0, n), pl.ds(*col))
        return pltpu.make_async_copy(src.at[idx], dst.at[idx], sem)

    def step(at, p):
        at(1, p).wait()
        at(0, p + LAG).wait()
        at(1, p + LAG + LOOK0).start(priority=0)
        nxt = at(0, p + LAG + LOOK1)
        if nxt is not None:
            nxt.start(priority=1)

    acc = {name: {} for name in REGIONS}

    def matvec(piece, vec):
        name, r0, n, (t0, nt) = piece
        for r in range(r0, r0 + n):
            w = bufs[name][1][r, t0:t0 + nt].astype(f32)
            for t in range(nt):
                kt, ct = divmod(r * REGIONS[name][1] + t0 + t, COL_TILES[name])
                _accumulate(acc[name], ct, w[t] * vec[kt * 8:kt * 8 + 8, :])

    def pre_at(odd, p):
        return copy(odd, p, PRE[2 * (p + N_PRE) + odd] if p < 0 else HEAD[2 * p + odd], 0)

    small = [pltpu.make_async_copy(x_hbm, x_v, sem_small.at[0]),
             pltpu.make_async_copy(gw_hbm, gw_v, sem_small.at[1]),
             pltpu.make_async_copy(wr_hbm, wr_v, sem_small.at[2])]
    per = (LAG + LOOK1) // LOOK0
    assert per * LOOK0 == LAG + LOOK1
    for i in range(LOOK0):
        for j in range(i * per, (i + 1) * per):
            pre_at(0, j - N_PRE).start(priority=1)
        pre_at(1, i - N_PRE).start(priority=0)
        wq_b[i, 200:] = jnp.zeros((56, 8, 128), bf16)
    for c in small:
        c.start()
    for i in range(LAG):
        pre_at(0, i - N_PRE).wait()
        pre_at(1, LOOK0 + i - N_PRE).start(priority=0)

    q_done = sum(piece[0] == 'q' for piece in PRE) // 2
    used = 0
    for i in range(N_PRE):
        step(pre_at, i - N_PRE)
        if i == X_STEP:
            for c in small:
                c.wait()
            x = x_v[0].astype(f32)
            gate = jax.nn.sigmoid(jnp.sum(x * gw_v[...].astype(f32).reshape(1, D), axis=-1, keepdims=True))
            rsel = jax.nn.sigmoid(jnp.sum(x * wr_v[...].astype(f32).reshape(1, D), axis=-1, keepdims=True))
            for j in range(0, D, 128):
                x_s[j:j + 128, :] = _column(x[:, j:j + 128])
        elif i > X_STEP:
            upto = min(used + 3, 2 * i + 2)
            for piece in PRE[used:upto]:
                if piece[0] != 'd':
                    matvec(piece, x_s)
            used = upto
        if i >= q_done and (i - q_done) % 10 == 0:
            assert used >= 2 * q_done
            for ct in range((i - q_done) // 10 * 4, (i - q_done) // 10 * 4 + 4):
                q_s[ct * 128:(ct + 1) * 128, :] = _column(_rowsum(acc['q'].pop(ct)))
    assert used == len(PRE) and not acc['q']

    def head(h, following, extra=None):
        def at(odd, p):
            if p < N_HEAD:
                return copy(odd, p, HEAD[2 * p + odd], h)
            return copy(odd, p, following[2 * (p - N_HEAD) + odd], h + 1)

        s, e, o, stat = {}, {}, {}, {}
        missing = {c: DH // 8 for c in range(0, W, KC)}
        for p in range(N_HEAD):
            step(at, p)
            for name, g0, n, (half, c) in HEAD[2 * p:2 * p + 2]:
                rows, cols = slice(half * 8, half * 8 + 8), slice(c, c + KC)
                if name == 'k':
                    for g in range(g0, g0 + n):
                        r0 = h * DH + g * 16 + half * 8
                        q = q_s[pl.ds(r0 if isinstance(r0, int) else pl.multiple_of(r0, 8), 8), :]
                        _accumulate(s, c, k_b[g, rows, cols].astype(f32) * jnp.tile(q, (1, KC // 128)))
                    missing[c] -= n
                    if missing[c] == 0:
                        s[c] = jnp.broadcast_to(_rowsum(s[c]), (8, KC)) * DH ** -0.5
                        for j in range(0, KC, 128):
                            tile = s[c][:, j:j + 128]
                            stat['max'] = jnp.maximum(stat['max'], tile) if 'max' in stat else tile
                        if not any(missing.values()):
                            row_max = jnp.max(stat['max'], axis=-1, keepdims=True)
                else:
                    if c not in e:
                        e[c] = jnp.exp(s[c] - row_max)
                        for j in range(0, KC, 128):
                            _accumulate(stat, 'sum', e[c][:, j:j + 128])
                    for g in range(g0, g0 + n):
                        pv = v_b[g, rows, cols].astype(f32) * e[c]
                        parts = [pv[:, j:j + 128] for j in range(0, KC, 128)]
                        while len(parts) > 1:
                            parts = [a + b for a, b in zip(parts[::2], parts[1::2])]
                        _accumulate(o, g * 16 + half * 8, parts[0])
            if extra is not None:
                extra(p)
        inv = 1.0 / jnp.sum(stat['sum'], axis=-1, keepdims=True)
        for r in range(0, DH, 8):
            r0 = h * DH + r
            o_s[pl.ds(r0 if isinstance(r0, int) else pl.multiple_of(r0, 8), 8), :] = jnp.broadcast_to(
                jnp.sum(o[r], axis=-1, keepdims=True) * inv, (8, 128))

    down = [piece for piece in PRE if piece[0] == 'd']

    def ffn(p):
        if p in (4, 10, 16):
            for ct in range(p // 6 * 4, p // 6 * 4 + 4):
                hidden = jax.nn.silu(_rowsum(acc['g'][ct])) * _rowsum(acc['u'][ct])
                h_s[ct * 128:(ct + 1) * 128, :] = _column(hidden)
        elif p > 16:
            for piece in down[(p - 17) * 2:(p - 16) * 2]:
                matvec(piece, h_s)

    assert 17 + len(down) // 2 <= N_HEAD
    jax.lax.fori_loop(0, H - 1, lambda h, _: head(h, HEAD), None)
    head(H - 1, POST, ffn)

    def post_at(odd, p):
        return copy(odd, p, POST[2 * p + odd]) if p < N_POST else None

    y = _rowsum(jnp.concatenate([acc['d'][ct] for ct in range(D // 128)], axis=1))
    b = (1.0 - gate) * (x + (x * 0.0 + y * rsel))
    n_issue = N_POST - LAG - LOOK0
    for p in range(N_POST):
        if p < n_issue:
            step(post_at, p)
        for odd in (1, 0):
            if p >= n_issue + (0 if odd else LAG):
                post_at(odd, p).wait()
            matvec(POST[2 * p + odd], o_s)
    a = _rowsum(jnp.concatenate([acc['o'][ct] for ct in range(D // 128)], axis=1))
    out_ref[0] = (gate * a + b).astype(bf16)


def _tiles(w, name):
    r, c = w.shape
    return w.reshape(r // 8, 8, c // 128, 128).transpose(0, 2, 1, 3).reshape(*REGIONS[name], 8, 128)


@jax.jit
def pallas_gated_mix__sliding_block_cached__moe_arch_mod__decode_kernel(
        A_x, A_k_cache, A_v_cache, A_wq, A_wo, B_x, B_w_r, B_w_gate, B_w_up, B_w_down, gate_w):
    del B_x
    kT = jnp.swapaxes(A_k_cache, 2, 3).reshape(H, DH // 16, 16, SK)
    vT = jnp.swapaxes(A_v_cache, 2, 3).reshape(H, DH // 16, 16, SK)
    vmem = pltpu.VMEM
    return pl.pallas_call(
        _kernel,
        out_shape=jax.ShapeDtypeStruct((1, 1, D), bf16),
        in_specs=[pl.BlockSpec(memory_space=pl.ANY)] * 10,
        out_specs=pl.BlockSpec(memory_space=pltpu.VMEM),
        scratch_shapes=[
            vmem((1, 1, D), bf16), vmem((D,), bf16), vmem((D,), bf16),
            vmem((DH // 16, 16, W), bf16), vmem((DH // 16, 16, W), bf16),
            *[vmem((*REGIONS[name], 8, 128), bf16) for name in 'qogud'],
            vmem((D, 128), f32), vmem((H * DH, 128), f32), vmem((F, 128), f32), vmem((H * DH, 128), f32),
            pltpu.SemaphoreType.DMA((NSEM,)), pltpu.SemaphoreType.DMA((NSEM,)),
            pltpu.SemaphoreType.DMA((3,)),
        ],
        compiler_params=pltpu.CompilerParams(
            vmem_limit_bytes=64 * 1024 * 1024,
            disable_semaphore_checks=True,
            disable_bounds_checks=True,
        ),
        name="gated_mix_decode",
    )(A_x, kT, vT, _tiles(A_wq, 'q'), _tiles(A_wo, 'o'), B_w_r,
      _tiles(B_w_gate, 'g'), _tiles(B_w_up, 'u'), _tiles(B_w_down, 'd'), gate_w)
```

```python
import jax
import jax.numpy as jnp
import jax.experimental.pallas as pl
import jax.experimental.pallas.tpu as pltpu

H, DH, SK, D, F = 32, 192, 32768, 640, 1536
W = min(4096, max(256, SK // 4))
BASE = SK - W

LOOK1, LOOK0 = 32, 12
LAG = 4
NSEM = 64
X_STEP = 16

f32 = jnp.float32
bf16 = jnp.bfloat16

REGIONS = dict(q=(15, 256), o=(15, 256), g=(4, 240), u=(4, 240), d=(4, 240))
COL_TILES = dict(q=H * DH // 128, o=D // 128, g=F // 128, u=F // 128, d=D // 128)
TW = 4
KC = 1024


def _sweep(*split):
    return [(name, r0, n, (t, TW)) for t in range(0, REGIONS[split[0][0]][1], TW) for name, r0, n in split]


def _kv_sweep(name, runs):
    return [(name, g + dg, n, (half, col * KC))
            for half, col in runs for g in range(0, DH // 16, 3) for dg, n in ((0, 2), (2, 1))]


_SPLIT15 = ((0, 3), (3, 2), (5, 4), (9, 2), (11, 3), (14, 1))
PRE = (_sweep(*[('q', r0, n) for r0, n in _SPLIT15])
       + _sweep(('g', 0, 4), ('u', 0, 2), ('d', 0, 4), ('u', 2, 2)))
HEAD = (_kv_sweep('k', ((0, 1), (0, 0), (1, 0), (1, 1), (0, 3), (0, 2), (1, 2), (1, 3)))
        + _kv_sweep('v', ((0, 0), (0, 1), (0, 2), (1, 0), (1, 1), (1, 2), (0, 3), (1, 3))))
POST = ([p for p in _sweep(*[('o', r0, n) for r0, n in _SPLIT15]) if p[1] < 11 or p[3][0] < 208]
        + [('o', r, 1, (t, 12)) for r in range(11, 15) for t in range(208, 256, 12)])
N_PRE, N_HEAD, N_POST = len(PRE) // 2, len(HEAD) // 2, len(POST) // 2
assert N_HEAD % NSEM == 0 and LOOK0 <= LOOK1 and LAG + LOOK1 < min(NSEM, N_HEAD)


def _rowsum(v):
    return jnp.sum(v, axis=0, keepdims=True)


def _column(row):
    return jnp.broadcast_to(row, (128, 128)).T


def _accumulate(acc, key, part):
    acc[key] = acc[key] + part if key in acc else part


def _kernel(x_hbm, kT, vT, wq, wo, wr_hbm, wg, wu, wd, gw_hbm, out_ref,
            x_v, wr_v, gw_v, k_b, v_b, wq_b, wo_b, wg_b, wu_b, wd_b,
            x_s, q_s, h_s, o_s, sem1, sem0, sem_small):
    bufs = dict(k=(kT, k_b), v=(vT, v_b), q=(wq, wq_b), o=(wo, wo_b),
                g=(wg, wg_b), u=(wu, wu_b), d=(wd, wd_b))

    def copy(odd, pos, piece, h=None):
        name, r0, n, col = piece
        src, dst = bufs[name]
        sem = (sem1, sem0)[odd].at[pos % NSEM]
        if name in 'kv':
            half, c = col
            return pltpu.make_async_copy(src.at[h, pl.ds(r0, n), pl.ds(half, 1), :, pl.ds(BASE + c, KC)],
                                         dst.at[pl.ds(r0, n), pl.ds(half, 1), :, pl.ds(c, KC)], sem)
        idx = (pl.ds(r0, n), pl.ds(*col))
        return pltpu.make_async_copy(src.at[idx], dst.at[idx], sem)

    def step(at, p):
        at(1, p).wait()
        at(0, p + LAG).wait()
        at(1, p + LAG + LOOK0).start(priority=0)
        nxt = at(0, p + LAG + LOOK1)
        if nxt is not None:
            nxt.start(priority=1)

    acc = {name: {} for name in REGIONS}

    def matvec(piece, vec):
        name, r0, n, (t0, nt) = piece
        for r in range(r0, r0 + n):
            w = bufs[name][1][r, t0:t0 + nt].astype(f32)
            for t in range(nt):
                kt, ct = divmod(r * REGIONS[name][1] + t0 + t, COL_TILES[name])
                _accumulate(acc[name], ct, w[t] * vec[kt * 8:kt * 8 + 8, :])

    def pre_at(odd, p):
        return copy(odd, p, PRE[2 * (p + N_PRE) + odd] if p < 0 else HEAD[2 * p + odd], 0)

    small = [pltpu.make_async_copy(x_hbm, x_v, sem_small.at[0]),
             pltpu.make_async_copy(gw_hbm, gw_v, sem_small.at[1]),
             pltpu.make_async_copy(wr_hbm, wr_v, sem_small.at[2])]
    per = (LAG + LOOK1) // LOOK0
    assert per * LOOK0 == LAG + LOOK1
    for i in range(LOOK0):
        for j in range(i * per, (i + 1) * per):
            pre_at(0, j - N_PRE).start(priority=1)
        pre_at(1, i - N_PRE).start(priority=0)
        wq_b[i, 200:] = jnp.zeros((56, 8, 128), bf16)
    for c in small:
        c.start()
    for i in range(LAG):
        pre_at(0, i - N_PRE).wait()
        pre_at(1, LOOK0 + i - N_PRE).start(priority=0)

    q_done = sum(piece[0] == 'q' for piece in PRE) // 2
    used = 0
    for i in range(N_PRE):
        step(pre_at, i - N_PRE)
        if i == X_STEP:
            for c in small:
                c.wait()
            x = x_v[0].astype(f32)
            gate = jax.nn.sigmoid(jnp.sum(x * gw_v[...].astype(f32).reshape(1, D), axis=-1, keepdims=True))
            rsel = jax.nn.sigmoid(jnp.sum(x * wr_v[...].astype(f32).reshape(1, D), axis=-1, keepdims=True))
            for j in range(0, D, 128):
                x_s[j:j + 128, :] = _column(x[:, j:j + 128])
        elif i > X_STEP:
            upto = min(used + 3, 2 * i + 2)
            for piece in PRE[used:upto]:
                if piece[0] != 'd':
                    matvec(piece, x_s)
            used = upto
        if i >= q_done and (i - q_done) % 10 == 0:
            assert used >= 2 * q_done
            for ct in range((i - q_done) // 10 * 4, (i - q_done) // 10 * 4 + 4):
                q_s[ct * 128:(ct + 1) * 128, :] = _column(_rowsum(acc['q'].pop(ct)))
    assert used == len(PRE) and not acc['q']

    def head(h, following, extra=None):
        def at(odd, p):
            if p < N_HEAD:
                return copy(odd, p, HEAD[2 * p + odd], h)
            return copy(odd, p, following[2 * (p - N_HEAD) + odd], h + 1)

        s, e, o, stat = {}, {}, {}, {}
        missing = {c: DH // 8 for c in range(0, W, KC)}
        for p in range(N_HEAD):
            step(at, p)
            for name, g0, n, (half, c) in HEAD[2 * p:2 * p + 2]:
                if name == 'k':
                    for g in range(g0, g0 + n):
                        r0 = h * DH + g * 16 + half * 8
                        q = q_s[pl.ds(r0 if isinstance(r0, int) else pl.multiple_of(r0, 8), 8), :]
                        q = jnp.concatenate([q] * (KC // 128), axis=1)
                        _accumulate(s, c, k_b[g, half, :, c:c + KC].astype(f32) * q)
                    missing[c] -= n
                    if missing[c] == 0:
                        s[c] = jnp.broadcast_to(_rowsum(s[c]), (8, KC)) * DH ** -0.5
                        for j in range(0, KC, 128):
                            tile = s[c][:, j:j + 128]
                            stat['max'] = jnp.maximum(stat['max'], tile) if 'max' in stat else tile
                        if not any(missing.values()):
                            row_max = jnp.max(stat['max'], axis=-1, keepdims=True)
                else:
                    if c not in e:
                        e[c] = jnp.exp(s[c] - row_max)
                        for j in range(0, KC, 128):
                            _accumulate(stat, 'sum', e[c][:, j:j + 128])
                    for g in range(g0, g0 + n):
                        pv = v_b[g, half, :, c:c + KC].astype(f32) * e[c]
                        parts = [pv[:, j:j + 128] for j in range(0, KC, 128)]
                        while len(parts) > 1:
                            parts = [a + b for a, b in zip(parts[::2], parts[1::2])]
                        _accumulate(o, g * 16 + half * 8, parts[0])
            if extra is not None:
                extra(p)
        inv = 1.0 / jnp.sum(stat['sum'], axis=-1, keepdims=True)
        for r in range(0, DH, 8):
            r0 = h * DH + r
            o_s[pl.ds(r0 if isinstance(r0, int) else pl.multiple_of(r0, 8), 8), :] = jnp.broadcast_to(
                jnp.sum(o[r], axis=-1, keepdims=True) * inv, (8, 128))

    down = [piece for piece in PRE if piece[0] == 'd']

    def ffn(p):
        if p in (4, 10, 16):
            for ct in range(p // 6 * 4, p // 6 * 4 + 4):
                hidden = jax.nn.silu(_rowsum(acc['g'][ct])) * _rowsum(acc['u'][ct])
                h_s[ct * 128:(ct + 1) * 128, :] = _column(hidden)
        elif p > 16:
            for piece in down[(p - 17) * 2:(p - 16) * 2]:
                matvec(piece, h_s)

    assert 17 + len(down) // 2 <= N_HEAD
    jax.lax.fori_loop(0, H - 1, lambda h, _: head(h, HEAD), None)
    head(H - 1, POST, ffn)

    def post_at(odd, p):
        return copy(odd, p, POST[2 * p + odd]) if p < N_POST else None

    y = _rowsum(jnp.concatenate([acc['d'][ct] for ct in range(D // 128)], axis=1))
    b = (1.0 - gate) * (x + (x * 0.0 + y * rsel))
    n_issue = N_POST - LAG - LOOK0
    for p in range(N_POST):
        if p < n_issue:
            step(post_at, p)
        for odd in (1, 0):
            if p >= n_issue + (0 if odd else LAG):
                post_at(odd, p).wait()
            matvec(POST[2 * p + odd], o_s)
    a = _rowsum(jnp.concatenate([acc['o'][ct] for ct in range(D // 128)], axis=1))
    out_ref[0] = (gate * a + b).astype(bf16)


def _tiles(w, name):
    r, c = w.shape
    return w.reshape(r // 8, 8, c // 128, 128).transpose(0, 2, 1, 3).reshape(*REGIONS[name], 8, 128)


@jax.jit
def pallas_gated_mix__sliding_block_cached__moe_arch_mod__decode_kernel(
        A_x, A_k_cache, A_v_cache, A_wq, A_wo, B_x, B_w_r, B_w_gate, B_w_up, B_w_down, gate_w):
    del B_x
    kT = jnp.swapaxes(A_k_cache, 2, 3).reshape(H, DH // 16, 2, 8, SK)
    vT = jnp.swapaxes(A_v_cache, 2, 3).reshape(H, DH // 16, 2, 8, SK)
    vmem = pltpu.VMEM
    return pl.pallas_call(
        _kernel,
        out_shape=jax.ShapeDtypeStruct((1, 1, D), bf16),
        in_specs=[pl.BlockSpec(memory_space=pl.ANY)] * 10,
        out_specs=pl.BlockSpec(memory_space=pltpu.VMEM),
        scratch_shapes=[
            vmem((1, 1, D), bf16), vmem((D,), bf16), vmem((D,), bf16),
            vmem((DH // 16, 2, 8, W), bf16), vmem((DH // 16, 2, 8, W), bf16),
            *[vmem((*REGIONS[name], 8, 128), bf16) for name in 'qogud'],
            vmem((D, 128), f32), vmem((H * DH, 128), f32), vmem((F, 128), f32), vmem((H * DH, 128), f32),
            pltpu.SemaphoreType.DMA((NSEM,)), pltpu.SemaphoreType.DMA((NSEM,)),
            pltpu.SemaphoreType.DMA((3,)),
        ],
        compiler_params=pltpu.CompilerParams(
            vmem_limit_bytes=64 * 1024 * 1024,
            disable_semaphore_checks=True,
            disable_bounds_checks=True,
        ),
        name="gated_mix_decode",
    )(A_x, kT, vT, _tiles(A_wq, 'q'), _tiles(A_wo, 'o'), B_w_r,
      _tiles(B_w_gate, 'g'), _tiles(B_w_up, 'u'), _tiles(B_w_down, 'd'), gate_w)
```

```python
import jax
import jax.numpy as jnp
import jax.experimental.pallas as pl
import jax.experimental.pallas.tpu as pltpu

H, DH, SK, D, F = 32, 192, 32768, 640, 1536
W = min(4096, max(256, SK // 4))
BASE = SK - W

LOOK1, LOOK0 = 41, 15
LAG = 4
NSEM = 80
X_STEP = 16

f32 = jnp.float32
bf16 = jnp.bfloat16

REGIONS = dict(q=(15, 256), o=(15, 256), g=(4, 240), u=(4, 240), d=(4, 240))
COL_TILES = dict(q=H * DH // 128, o=D // 128, g=F // 128, u=F // 128, d=D // 128)
TW = 4
KC = 1024


def _sweep(*split):
    return [(name, r0, n, (t, TW)) for t in range(0, REGIONS[split[0][0]][1], TW) for name, r0, n in split]


def _kv_sweep(name, runs):
    return [(name, g0, n, (half, col * KC)) for half, col in runs
            for g0, n in ((0, 2), (2, 1), (3, 1), (4, 1), (5, 2), (7, 1), (8, 1), (9, 1), (10, 1), (11, 1))]


_SPLIT15 = ((0, 3), (3, 2), (5, 4), (9, 2), (11, 3), (14, 1))
PRE = (_sweep(*[('q', r0, n) for r0, n in _SPLIT15])
       + _sweep(('g', 0, 4), ('u', 0, 2), ('d', 0, 4), ('u', 2, 2)))
HEAD = (_kv_sweep('k', ((0, 1), (0, 0), (1, 0), (1, 1), (0, 3), (0, 2), (1, 2), (1, 3)))
        + _kv_sweep('v', ((0, 0), (0, 1), (0, 2), (1, 0), (1, 1), (1, 2), (0, 3), (1, 3))))
POST = ([p for p in _sweep(*[('o', r0, n) for r0, n in _SPLIT15]) if p[1] < 11 or p[3][0] < 208]
        + [('o', r, 1, (t, 12)) for r in range(11, 15) for t in range(208, 256, 12)])
N_PRE, N_HEAD, N_POST = len(PRE) // 2, len(HEAD) // 2, len(POST) // 2
assert N_HEAD % NSEM == 0 and LOOK0 <= LOOK1 and LAG + LOOK1 < min(NSEM, N_HEAD)


def _rowsum(v):
    return jnp.sum(v, axis=0, keepdims=True)


def _column(row):
    return jnp.broadcast_to(row, (128, 128)).T


def _accumulate(acc, key, part):
    acc[key] = acc[key] + part if key in acc else part


def _kernel(x_hbm, kT, vT, wq, wo, wr_hbm, wg, wu, wd, gw_hbm, out_ref,
            x_v, wr_v, gw_v, k_b, v_b, wq_b, wo_b, wg_b, wu_b, wd_b,
            x_s, q_s, h_s, o_s, sem1, sem0, sem_small):
    bufs = dict(k=(kT, k_b), v=(vT, v_b), q=(wq, wq_b), o=(wo, wo_b),
                g=(wg, wg_b), u=(wu, wu_b), d=(wd, wd_b))

    def copy(odd, pos, piece, h=None):
        name, r0, n, col = piece
        src, dst = bufs[name]
        sem = (sem1, sem0)[odd].at[pos % NSEM]
        if name in 'kv':
            half, c = col
            return pltpu.make_async_copy(src.at[h, pl.ds(r0, n), pl.ds(half, 1), :, pl.ds(BASE + c, KC)],
                                         dst.at[pl.ds(r0, n), pl.ds(half, 1), :, pl.ds(c, KC)], sem)
        idx = (pl.ds(r0, n), pl.ds(*col))
        return pltpu.make_async_copy(src.at[idx], dst.at[idx], sem)

    def step(at, p):
        at(1, p).wait()
        at(0, p + LAG).wait()
        at(1, p + LAG + LOOK0).start(priority=0)
        nxt = at(0, p + LAG + LOOK1)
        if nxt is not None:
            nxt.start(priority=1)

    acc = {name: {} for name in REGIONS}

    def matvec(piece, vec):
        name, r0, n, (t0, nt) = piece
        for r in range(r0, r0 + n):
            w = bufs[name][1][r, t0:t0 + nt].astype(f32)
            for t in range(nt):
                kt, ct = divmod(r * REGIONS[name][1] + t0 + t, COL_TILES[name])
                _accumulate(acc[name], ct, w[t] * vec[kt * 8:kt * 8 + 8, :])

    def pre_at(odd, p):
        return copy(odd, p, PRE[2 * (p + N_PRE) + odd] if p < 0 else HEAD[2 * p + odd], 0)

    small = [pltpu.make_async_copy(x_hbm, x_v, sem_small.at[0]),
             pltpu.make_async_copy(gw_hbm, gw_v, sem_small.at[1]),
             pltpu.make_async_copy(wr_hbm, wr_v, sem_small.at[2])]
    per = (LAG + LOOK1) // LOOK0
    assert per * LOOK0 == LAG + LOOK1
    for i in range(LOOK0):
        for j in range(i * per, (i + 1) * per):
            pre_at(0, j - N_PRE).start(priority=1)
        pre_at(1, i - N_PRE).start(priority=0)
        wq_b[i, 200:] = jnp.zeros((56, 8, 128), bf16)
    for c in small:
        c.start()
    for i in range(LAG):
        pre_at(0, i - N_PRE).wait()
        pre_at(1, LOOK0 + i - N_PRE).start(priority=0)

    q_done = sum(piece[0] == 'q' for piece in PRE) // 2
    used = 0
    for i in range(N_PRE):
        step(pre_at, i - N_PRE)
        if i == X_STEP:
            for c in small:
                c.wait()
            x = x_v[0].astype(f32)
            gate = jax.nn.sigmoid(jnp.sum(x * gw_v[...].astype(f32).reshape(1, D), axis=-1, keepdims=True))
            rsel = jax.nn.sigmoid(jnp.sum(x * wr_v[...].astype(f32).reshape(1, D), axis=-1, keepdims=True))
            for j in range(0, D, 128):
                x_s[j:j + 128, :] = _column(x[:, j:j + 128])
        elif i > X_STEP:
            upto = min(used + 3, 2 * i + 2)
            for piece in PRE[used:upto]:
                if piece[0] != 'd':
                    matvec(piece, x_s)
            used = upto
        if i >= q_done and (i - q_done) % 10 == 0:
            assert used >= 2 * q_done
            for ct in range((i - q_done) // 10 * 4, (i - q_done) // 10 * 4 + 4):
                q_s[ct * 128:(ct + 1) * 128, :] = _column(_rowsum(acc['q'].pop(ct)))
    assert used == len(PRE) and not acc['q']

    def head(h, following, extra=None):
        def at(odd, p):
            if p < N_HEAD:
                return copy(odd, p, HEAD[2 * p + odd], h)
            return copy(odd, p, following[2 * (p - N_HEAD) + odd], h + 1)

        s, e, o, stat = {}, {}, {}, {}
        missing = {c: DH // 8 for c in range(0, W, KC)}
        for p in range(N_HEAD):
            step(at, p)
            for name, g0, n, (half, c) in HEAD[2 * p:2 * p + 2]:
                if name == 'k':
                    for g in range(g0, g0 + n):
                        r0 = h * DH + g * 16 + half * 8
                        q = q_s[pl.ds(r0 if isinstance(r0, int) else pl.multiple_of(r0, 8), 8), :]
                        q = jnp.concatenate([q] * (KC // 128), axis=1)
                        _accumulate(s, c, k_b[g, half, :, c:c + KC].astype(f32) * q)
                    missing[c] -= n
                    if missing[c] == 0:
                        s[c] = jnp.broadcast_to(_rowsum(s[c]), (8, KC)) * DH ** -0.5
                        for j in range(0, KC, 128):
                            tile = s[c][:, j:j + 128]
                            stat['max'] = jnp.maximum(stat['max'], tile) if 'max' in stat else tile
                        if not any(missing.values()):
                            row_max = jnp.max(stat['max'], axis=-1, keepdims=True)
                else:
                    if c not in e:
                        e[c] = jnp.exp(s[c] - row_max)
                        for j in range(0, KC, 128):
                            _accumulate(stat, 'sum', e[c][:, j:j + 128])
                    for g in range(g0, g0 + n):
                        pv = v_b[g, half, :, c:c + KC].astype(f32) * e[c]
                        parts = [pv[:, j:j + 128] for j in range(0, KC, 128)]
                        while len(parts) > 1:
                            parts = [a + b for a, b in zip(parts[::2], parts[1::2])]
                        _accumulate(o, g * 16 + half * 8, parts[0])
            if extra is not None:
                extra(p)
        inv = 1.0 / jnp.sum(stat['sum'], axis=-1, keepdims=True)
        for r in range(0, DH, 8):
            r0 = h * DH + r
            o_s[pl.ds(r0 if isinstance(r0, int) else pl.multiple_of(r0, 8), 8), :] = jnp.broadcast_to(
                jnp.sum(o[r], axis=-1, keepdims=True) * inv, (8, 128))

    down = [piece for piece in PRE if piece[0] == 'd']

    def ffn(p):
        if p in (4, 10, 16):
            for ct in range(p // 6 * 4, p // 6 * 4 + 4):
                hidden = jax.nn.silu(_rowsum(acc['g'][ct])) * _rowsum(acc['u'][ct])
                h_s[ct * 128:(ct + 1) * 128, :] = _column(hidden)
        elif p > 16:
            for piece in down[(p - 17) * 2:(p - 16) * 2]:
                matvec(piece, h_s)

    assert 17 + len(down) // 2 <= N_HEAD
    jax.lax.fori_loop(0, H - 1, lambda h, _: head(h, HEAD), None)
    head(H - 1, POST, ffn)

    def post_at(odd, p):
        return copy(odd, p, POST[2 * p + odd]) if p < N_POST else None

    y = _rowsum(jnp.concatenate([acc['d'][ct] for ct in range(D // 128)], axis=1))
    b = (1.0 - gate) * (x + (x * 0.0 + y * rsel))
    n_issue = N_POST - LAG - LOOK0
    for p in range(N_POST):
        if p < n_issue:
            step(post_at, p)
        for odd in (1, 0):
            if p >= n_issue + (0 if odd else LAG):
                post_at(odd, p).wait()
            matvec(POST[2 * p + odd], o_s)
    a = _rowsum(jnp.concatenate([acc['o'][ct] for ct in range(D // 128)], axis=1))
    out_ref[0] = (gate * a + b).astype(bf16)


def _tiles(w, name):
    r, c = w.shape
    return w.reshape(r // 8, 8, c // 128, 128).transpose(0, 2, 1, 3).reshape(*REGIONS[name], 8, 128)


@jax.jit
def pallas_gated_mix__sliding_block_cached__moe_arch_mod__decode_kernel(
        A_x, A_k_cache, A_v_cache, A_wq, A_wo, B_x, B_w_r, B_w_gate, B_w_up, B_w_down, gate_w):
    del B_x
    kT = jnp.swapaxes(A_k_cache, 2, 3).reshape(H, DH // 16, 2, 8, SK)
    vT = jnp.swapaxes(A_v_cache, 2, 3).reshape(H, DH // 16, 2, 8, SK)
    vmem = pltpu.VMEM
    return pl.pallas_call(
        _kernel,
        out_shape=jax.ShapeDtypeStruct((1, 1, D), bf16),
        in_specs=[pl.BlockSpec(memory_space=pl.ANY)] * 10,
        out_specs=pl.BlockSpec(memory_space=pltpu.VMEM),
        scratch_shapes=[
            vmem((1, 1, D), bf16), vmem((D,), bf16), vmem((D,), bf16),
            vmem((DH // 16, 2, 8, W), bf16), vmem((DH // 16, 2, 8, W), bf16),
            *[vmem((*REGIONS[name], 8, 128), bf16) for name in 'qogud'],
            vmem((D, 128), f32), vmem((H * DH, 128), f32), vmem((F, 128), f32), vmem((H * DH, 128), f32),
            pltpu.SemaphoreType.DMA((NSEM,)), pltpu.SemaphoreType.DMA((NSEM,)),
            pltpu.SemaphoreType.DMA((3,)),
        ],
        compiler_params=pltpu.CompilerParams(
            vmem_limit_bytes=64 * 1024 * 1024,
            disable_semaphore_checks=True,
            disable_bounds_checks=True,
        ),
        name="gated_mix_decode",
    )(A_x, kT, vT, _tiles(A_wq, 'q'), _tiles(A_wo, 'o'), B_w_r,
      _tiles(B_w_gate, 'g'), _tiles(B_w_up, 'u'), _tiles(B_w_down, 'd'), gate_w)
```

```python
import jax
import jax.numpy as jnp
import jax.experimental.pallas as pl
import jax.experimental.pallas.tpu as pltpu

H, DH, SK, D, F = 32, 192, 32768, 640, 1536
W = min(4096, max(256, SK // 4))
BASE = SK - W

LOOK1, LOOK0 = 41, 15
LAG = 4
NSEM = 80
X_STEP = 16

f32 = jnp.float32
bf16 = jnp.bfloat16

REGIONS = dict(q=(15, 256), o=(15, 256), g=(4, 240), u=(4, 240), d=(4, 240))
COL_TILES = dict(q=H * DH // 128, o=D // 128, g=F // 128, u=F // 128, d=D // 128)
TW = 4
KC = 1024


def _sweep(*split):
    return [(name, r0, n, (t, TW)) for t in range(0, REGIONS[split[0][0]][1], TW) for name, r0, n in split]


def _kv_sweep(name, runs):
    return [(name, g0, n, (half, col * KC)) for half, col in runs
            for g0, n in ((0, 2), (2, 1), (3, 1), (4, 1), (5, 2), (7, 1), (8, 1), (9, 1), (10, 1), (11, 1))]


_SPLIT15 = ((0, 3), (3, 2), (5, 4), (9, 2), (11, 3), (14, 1))
PRE = (_sweep(*[('q', r0, n) for r0, n in _SPLIT15])
       + _sweep(('g', 0, 4), ('u', 0, 2), ('d', 0, 4), ('u', 2, 2)))
HEAD = (_kv_sweep('k', ((0, 1), (0, 0), (1, 0), (1, 1), (0, 3), (0, 2), (1, 2), (1, 3)))
        + _kv_sweep('v', ((0, 0), (0, 1), (0, 2), (1, 0), (1, 1), (1, 2), (0, 3), (1, 3))))
POST = ([p for p in _sweep(*[('o', r0, n) for r0, n in _SPLIT15]) if p[1] < 11 or p[3][0] < 208]
        + [('o', r, 1, (t, 12)) for r in range(11, 15) for t in range(208, 256, 12)])
N_PRE, N_HEAD, N_POST = len(PRE) // 2, len(HEAD) // 2, len(POST) // 2
assert N_HEAD % NSEM == 0 and LOOK0 <= LOOK1 and LAG + LOOK1 < min(NSEM, N_HEAD)


def _rowsum(v):
    return jnp.sum(v, axis=0, keepdims=True)


def _column(row):
    return jnp.broadcast_to(row, (128, 128)).T


def _fold(op, v):
    while v.shape[1] > 128:
        v = op(v[:, :v.shape[1] // 2], v[:, v.shape[1] // 2:])
    return v


def _accumulate(acc, key, part):
    acc[key] = acc[key] + part if key in acc else part


def _kernel(x_hbm, kT, vT, wq, wo, wr_hbm, wg, wu, wd, gw_hbm, out_ref,
            x_v, wr_v, gw_v, k_b, v_b, wq_b, wo_b, wg_b, wu_b, wd_b,
            x_s, q_s, h_s, o_s, sem1, sem0, sem_small):
    bufs = dict(k=(kT, k_b), v=(vT, v_b), q=(wq, wq_b), o=(wo, wo_b),
                g=(wg, wg_b), u=(wu, wu_b), d=(wd, wd_b))

    def copy(odd, pos, piece, h=None):
        name, r0, n, col = piece
        src, dst = bufs[name]
        sem = (sem1, sem0)[odd].at[pos % NSEM]
        if name in 'kv':
            half, c = col
            return pltpu.make_async_copy(src.at[h, pl.ds(r0, n), pl.ds(half, 1), :, pl.ds(BASE + c, KC)],
                                         dst.at[pl.ds(r0, n), pl.ds(half, 1), :, pl.ds(c, KC)], sem)
        idx = (pl.ds(r0, n), pl.ds(*col))
        return pltpu.make_async_copy(src.at[idx], dst.at[idx], sem)

    def step(at, p):
        at(1, p).wait()
        at(0, p + LAG).wait()
        at(1, p + LAG + LOOK0).start(priority=0)
        nxt = at(0, p + LAG + LOOK1)
        if nxt is not None:
            nxt.start(priority=1)

    acc = {name: {} for name in REGIONS}

    def matvec(piece, vec):
        name, r0, n, (t0, nt) = piece
        for r in range(r0, r0 + n):
            w = bufs[name][1][r, t0:t0 + nt].astype(f32)
            t = 0
            while t < nt:
                kt, ct = divmod(r * REGIONS[name][1] + t0 + t, COL_TILES[name])
                m = min(nt - t, COL_TILES[name] - ct)
                prod = w[t:t + m] * vec[kt * 8:kt * 8 + 8, :]
                if COL_TILES[name] % TW == 0:
                    _accumulate(acc[name], ct, prod)
                else:
                    for j in range(m):
                        _accumulate(acc[name], ct + j, prod[j])
                t += m

    def pre_at(odd, p):
        return copy(odd, p, PRE[2 * (p + N_PRE) + odd] if p < 0 else HEAD[2 * p + odd], 0)

    small = [pltpu.make_async_copy(x_hbm, x_v, sem_small.at[0]),
             pltpu.make_async_copy(gw_hbm, gw_v, sem_small.at[1]),
             pltpu.make_async_copy(wr_hbm, wr_v, sem_small.at[2])]
    per = (LAG + LOOK1) // LOOK0
    assert per * LOOK0 == LAG + LOOK1
    for i in range(LOOK0):
        for j in range(i * per, (i + 1) * per):
            pre_at(0, j - N_PRE).start(priority=1)
        pre_at(1, i - N_PRE).start(priority=0)
        wq_b[i, 200:] = jnp.zeros((56, 8, 128), bf16)
    for c in small:
        c.start()
    for i in range(LAG):
        pre_at(0, i - N_PRE).wait()
        pre_at(1, LOOK0 + i - N_PRE).start(priority=0)

    q_done = sum(piece[0] == 'q' for piece in PRE) // 2
    used = 0
    for i in range(N_PRE):
        step(pre_at, i - N_PRE)
        if i == X_STEP:
            for c in small:
                c.wait()
            x = x_v[0].astype(f32)
            gate = jax.nn.sigmoid(jnp.sum(x * gw_v[...].astype(f32).reshape(1, D), axis=-1, keepdims=True))
            rsel = jax.nn.sigmoid(jnp.sum(x * wr_v[...].astype(f32).reshape(1, D), axis=-1, keepdims=True))
            for j in range(0, D, 128):
                x_s[j:j + 128, :] = _column(x[:, j:j + 128])
        elif i > X_STEP:
            upto = min(used + 3, 2 * i + 2)
            for piece in PRE[used:upto]:
                if piece[0] != 'd':
                    matvec(piece, x_s)
            used = upto
        if i >= q_done and (i - q_done) % 10 == 0:
            assert used >= 2 * q_done
            ct = (i - q_done) // 10 * TW
            q = acc['q'].pop(ct)
            for j in range(TW):
                q_s[(ct + j) * 128:(ct + j + 1) * 128, :] = _column(_rowsum(q[j]))
    assert used == len(PRE) and not acc['q']

    def head(h, following, extra=None):
        def at(odd, p):
            if p < N_HEAD:
                return copy(odd, p, HEAD[2 * p + odd], h)
            return copy(odd, p, following[2 * (p - N_HEAD) + odd], h + 1)

        s, e, o, stat = {}, {}, {}, {}
        missing = {c: DH // 8 for c in range(0, W, KC)}
        for p in range(N_HEAD):
            step(at, p)
            for name, g0, n, (half, c) in HEAD[2 * p:2 * p + 2]:
                if name == 'k':
                    for g in range(g0, g0 + n):
                        r0 = h * DH + g * 16 + half * 8
                        q = q_s[pl.ds(r0 if isinstance(r0, int) else pl.multiple_of(r0, 8), 8), :]
                        q = jnp.concatenate([q] * (KC // 128), axis=1)
                        _accumulate(s, c, k_b[g, half, :, c:c + KC].astype(f32) * q)
                    missing[c] -= n
                    if missing[c] == 0:
                        s[c] = jnp.broadcast_to(_rowsum(s[c]), (8, KC)) * DH ** -0.5
                        top = _fold(jnp.maximum, s[c])
                        stat['max'] = jnp.maximum(stat['max'], top) if 'max' in stat else top
                        if not any(missing.values()):
                            row_max = jnp.max(stat['max'], axis=-1, keepdims=True)
                else:
                    if c not in e:
                        e[c] = jnp.exp(s[c] - row_max)
                        _accumulate(stat, 'sum', _fold(jnp.add, e[c]))
                    for g in range(g0, g0 + n):
                        pv = v_b[g, half, :, c:c + KC].astype(f32) * e[c]
                        _accumulate(o, g * 16 + half * 8, _fold(jnp.add, pv))
            if extra is not None:
                extra(p)
        inv = 1.0 / jnp.sum(stat['sum'], axis=-1, keepdims=True)
        for r in range(0, DH, 8):
            r0 = h * DH + r
            o_s[pl.ds(r0 if isinstance(r0, int) else pl.multiple_of(r0, 8), 8), :] = jnp.broadcast_to(
                jnp.sum(o[r], axis=-1, keepdims=True) * inv, (8, 128))

    down = [piece for piece in PRE if piece[0] == 'd']

    def ffn(p):
        if p in (4, 10, 16):
            ct = p // 6 * TW
            for j in range(TW):
                hidden = jax.nn.silu(_rowsum(acc['g'][ct][j])) * _rowsum(acc['u'][ct][j])
                h_s[(ct + j) * 128:(ct + j + 1) * 128, :] = _column(hidden)
        elif p > 16:
            for piece in down[(p - 17) * 2:(p - 16) * 2]:
                matvec(piece, h_s)

    assert 17 + len(down) // 2 <= N_HEAD
    jax.lax.fori_loop(0, H - 1, lambda h, _: head(h, HEAD), None)
    head(H - 1, POST, ffn)

    def post_at(odd, p):
        return copy(odd, p, POST[2 * p + odd]) if p < N_POST else None

    y = _rowsum(jnp.concatenate([acc['d'][ct] for ct in range(D // 128)], axis=1))
    b = (1.0 - gate) * (x + (x * 0.0 + y * rsel))
    n_issue = N_POST - LAG - LOOK0
    for p in range(N_POST):
        if p < n_issue:
            step(post_at, p)
        for odd in (1, 0):
            if p >= n_issue + (0 if odd else LAG):
                post_at(odd, p).wait()
            matvec(POST[2 * p + odd], o_s)
    a = _rowsum(jnp.concatenate([acc['o'][ct] for ct in range(D // 128)], axis=1))
    out_ref[0] = (gate * a + b).astype(bf16)


def _tiles(w, name):
    r, c = w.shape
    return w.reshape(r // 8, 8, c // 128, 128).transpose(0, 2, 1, 3).reshape(*REGIONS[name], 8, 128)


@jax.jit
def pallas_gated_mix__sliding_block_cached__moe_arch_mod__decode_kernel(
        A_x, A_k_cache, A_v_cache, A_wq, A_wo, B_x, B_w_r, B_w_gate, B_w_up, B_w_down, gate_w):
    del B_x
    kT = jnp.swapaxes(A_k_cache, 2, 3).reshape(H, DH // 16, 2, 8, SK)
    vT = jnp.swapaxes(A_v_cache, 2, 3).reshape(H, DH // 16, 2, 8, SK)
    vmem = pltpu.VMEM
    return pl.pallas_call(
        _kernel,
        out_shape=jax.ShapeDtypeStruct((1, 1, D), bf16),
        in_specs=[pl.BlockSpec(memory_space=pl.ANY)] * 10,
        out_specs=pl.BlockSpec(memory_space=pltpu.VMEM),
        scratch_shapes=[
            vmem((1, 1, D), bf16), vmem((D,), bf16), vmem((D,), bf16),
            vmem((DH // 16, 2, 8, W), bf16), vmem((DH // 16, 2, 8, W), bf16),
            *[vmem((*REGIONS[name], 8, 128), bf16) for name in 'qogud'],
            vmem((D, 128), f32), vmem((H * DH, 128), f32), vmem((F, 128), f32), vmem((H * DH, 128), f32),
            pltpu.SemaphoreType.DMA((NSEM,)), pltpu.SemaphoreType.DMA((NSEM,)),
            pltpu.SemaphoreType.DMA((3,)),
        ],
        compiler_params=pltpu.CompilerParams(
            vmem_limit_bytes=64 * 1024 * 1024,
            disable_semaphore_checks=True,
            disable_bounds_checks=True,
        ),
        name="gated_mix_decode",
    )(A_x, kT, vT, _tiles(A_wq, 'q'), _tiles(A_wo, 'o'), B_w_r,
      _tiles(B_w_gate, 'g'), _tiles(B_w_up, 'u'), _tiles(B_w_down, 'd'), gate_w)
```
